```python
import jax
import jax.numpy as jnp

def _softmax(x, axis=-1):
    return jax.nn.softmax(x, axis=axis)
def _gelu(x):
    return jax.nn.gelu(x, approximate=True)
def _silu(x):
    return jax.nn.silu(x)
def _sigmoid(x):
    return jax.nn.sigmoid(x)
def _layernorm(x, axis=-1, eps=1e-5):
    m = jnp.mean(x, axis=axis, keepdims=True)
    v = jnp.var(x, axis=axis, keepdims=True)
    return (x - m) / jnp.sqrt(v + eps)
def _scatter_add(tgt, idx, src, axis=0):
    return tgt.at[idx].add(src)
def _segment_sum(src, seg, n):
    return jax.ops.segment_sum(src, seg, n)
class _Rng:
    def __init__(self, key):
        self._k = key
    def _next(self):
        self._k, sub = jax.random.split(self._k)
        return sub
    def normal(self, shape):
        return jax.random.normal(self._next(), shape, dtype=jnp.bfloat16)
    def randint(self, lo, hi, shape):
        return jax.random.randint(self._next(), shape, lo, hi, dtype=jnp.int32)
    def uniform(self, shape, lo=0.0, hi=1.0):
        return jax.random.uniform(self._next(), shape, jnp.bfloat16, lo, hi)
    def permutation(self, n):
        return jax.random.permutation(self._next(), n)


kernel_name = 'concat_heads__mha_block_cached__compressed_kv_cla__decode'

def setup_inputs():
    _rng = _Rng(jax.random.key(int.from_bytes(__import__("os").urandom(4), "little")))
    _w = (lambda a: (lambda t: t.astype(jnp.bfloat16) if jnp.issubdtype(t.dtype, jnp.floating) else t)(jnp.asarray(a)))
    def _A_setup():
        B, Sq, D = 4, 1, 576
        H, Sk, Dh = 32, 4096, 128
        return {
            "x": _w((lambda *s: _rng.normal(s) * 0.05)(B, Sq, D)),
            "k_cache": _w((lambda *s: _rng.normal(s) * 0.05)(B, H, Sk, Dh)),
            "v_cache": _w((lambda *s: _rng.normal(s) * 0.05)(B, H, Sk, Dh)),
            "wq": _w((lambda *s: _rng.normal(s) * 0.05)(D, H * Dh) * (D ** -0.5)),
            "wo": _w((lambda *s: _rng.normal(s) * 0.05)(H * Dh, D) * ((H * Dh) ** -0.5)),
        }
    _A_in = _A_setup()

    def _B_setup():
        B, H, Sq, Sk, D, M = 4, 32, 1, 4096, 128, 576
        Dc = 4 * D
        return {
            "x": _w((lambda *s: _rng.normal(s) * 0.05)(B, Sq, M)),
            "c_kv": _w((lambda *s: _rng.normal(s) * 0.05)(B, Sk, Dc)),
            "w_q": _w((lambda *s: _rng.normal(s) * 0.05)(M, H, D) * (M ** -0.5)),
            "w_uk": _w((lambda *s: _rng.normal(s) * 0.05)(Dc, H, D) * (Dc ** -0.5)),
            "w_uv": _w((lambda *s: _rng.normal(s) * 0.05)(Dc, H, D) * (Dc ** -0.5)),
            "w_o": _w((lambda *s: _rng.normal(s) * 0.05)(H, D, M) * ((H * D) ** -0.5)),
        }
    _B_in = _B_setup()

    return {
        "A_x": _A_in["x"],
        "A_k_cache": _A_in["k_cache"],
        "A_v_cache": _A_in["v_cache"],
        "A_wq": _A_in["wq"],
        "A_wo": _A_in["wo"],
        "B_x": _B_in["x"],
        "B_c_kv": _B_in["c_kv"],
        "B_w_q": _B_in["w_q"],
        "B_w_uk": _B_in["w_uk"],
        "B_w_uv": _B_in["w_uv"],
        "B_w_o": _B_in["w_o"],
    }

def reference(A_x, A_k_cache, A_v_cache, A_wq, A_wo, B_x, B_c_kv, B_w_q, B_w_uk, B_w_uv, B_w_o):
    def _A_ref(x, k_cache, v_cache, wq, wo):
        B, Sq, D = x.shape
        H, Dh = 32, 128
        q = (lambda x, *d: x.transpose(*d))((x @ wq).reshape(B, Sq, H, Dh), 0, 2, 1, 3)
        scores = jnp.einsum("bhqd,bhkd->bhqk", q, k_cache) * (Dh ** -0.5)
        p = _softmax(scores, axis=-1)
        o = jnp.einsum("bhqk,bhkd->bhqd", p, v_cache)
        return (lambda x, *d: x.transpose(*d))(o, 0, 2, 1, 3).reshape(B, Sq, H * Dh) @ wo

    def _B_ref(x, c_kv, w_q, w_uk, w_uv, w_o):
        B, Sq, M = x.shape[0], x.shape[1], x.shape[2]
        Sk = c_kv.shape[1]
        H, D = w_q.shape[1], w_q.shape[2]
        q = jnp.einsum("bqm,mhd->bhqd", x, w_q)
        k = jnp.einsum("bkc,chd->bhkd", c_kv, w_uk)
        v = jnp.einsum("bkc,chd->bhkd", c_kv, w_uv)
        scores = jnp.einsum("bhqd,bhkd->bhqk", q, k) * (D ** -0.5)
        off = Sk - Sq
        qi = jnp.arange(Sq)[:, None]
        kj = jnp.arange(Sk)[None, :]
        cmask = kj <= (qi + off)
        scores = jnp.where(cmask[None, None], scores, -1e9)
        p = _softmax(scores, axis=-1)
        ctx = jnp.einsum("bhqk,bhkd->bhqd", p, v)
        return jnp.einsum("bhqd,hdm->bqm", ctx, w_o)

    a = _A_ref(A_x, A_k_cache, A_v_cache, A_wq, A_wo)
    b = _B_ref(B_x, B_c_kv, B_w_q, B_w_uk, B_w_uv, B_w_o)
    return jnp.concatenate([a, b], axis=-1)
```

```python
import jax
import jax.numpy as jnp
from jax import lax
import jax.experimental.pallas as pl
import jax.experimental.pallas.tpu as pltpu

F32 = jnp.float32
BF16 = jnp.bfloat16

NB = 4
NH = 32
SK = 4096
DH = 128
DM = 576
DC = 512
NSTEP = NB * NH
KV_SLOTS = 3
LOOK = KV_SLOTS - 1
LAG = 3
SCALE = DH ** -0.5

CHUNK = 4096
CKV_ROWS = 1024
WO_COLS = 1024
WOB_ROWS = 8 * DM

S_WO, N_WO = 0, 4
S_WQB, N_WQB = 4, 5
S_WUK, N_WUK = 9, 4
S_CKV, N_CKV = 13, 16
S_WUV, N_WUV = 29, 4
S_WOB, N_WOB = 33, 4
N_SIDE_SEMS = 4


def _pieces(nrows, piece):
    out, r = [], 0
    while r < nrows:
        n = min(piece, nrows - r)
        out.append((r, n))
        r += n
    return out


def _interleave(a, b):
    out = []
    for i in range(max(len(a), len(b))):
        if i < len(a):
            out.append(a[i])
        if i < len(b):
            out.append(b[i])
    return out


def _start_rows(src, dst, src_row0, dst_row0, nrows, piece, sem):
    ps = _pieces(nrows, piece)
    half = (len(ps) + 1) // 2
    first = [(p, 0) for p in ps[:half]]
    second = [(p, 1) for p in ps[half:]]
    for (r, n), prio in _interleave(first, second):
        pltpu.make_async_copy(src.at[pl.ds(src_row0 + r, n)], dst.at[pl.ds(dst_row0 + r, n)],
                              sem).start(priority=prio)


def _wait(buf_view, sem):
    pltpu.make_async_copy(buf_view, buf_view, sem).wait()


def _kernel(xa_hbm, k_hbm, v_hbm, wq_hbm, wo_hbm, xb_hbm, ckv_hbm, wqb_hbm, wuk_hbm, wuv_hbm,
            wob_hbm, out_ref,
            xa_v, xb_v, kbuf, vbuf, wq_v, wo_v, wqb_v, wuk_v, wuv_v, wob_v, ckv_v,
            p_v, x8_v, xbc_v, q_v, o_v, qb_v, qabs_v, m_v, l_v, acc_v, cl_v, ctx_v, cp_v,
            outa_v, outb_v,
            sem_x, sem_wq, sem_k, sem_v, sem_wo, sem_side):

    kv_pieces = _pieces(SK, 224)

    def start_kv(step, slot):
        h = step // NB
        b = step % NB
        for r, n in kv_pieces:
            pltpu.make_async_copy(k_hbm.at[b, h, pl.ds(r, n)], kbuf.at[slot, pl.ds(r, n)],
                                  sem_k.at[slot]).start(priority=0)
            pltpu.make_async_copy(v_hbm.at[b, h, pl.ds(r, n)], vbuf.at[slot, pl.ds(r, n)],
                                  sem_v.at[slot]).start(priority=1)

    pltpu.make_async_copy(xa_hbm, xa_v, sem_x.at[0]).start()
    pltpu.make_async_copy(xb_hbm, xb_v, sem_x.at[1]).start()
    ng = DM // 8
    for g in range(ng // 2):
        for c in range(2):
            for part in range(2):
                r0 = (g + part * (ng // 2)) * 8
                pltpu.make_async_copy(wq_hbm.at[pl.ds(r0, 8), pl.ds(c * 2048, 2048)],
                                      wq_v.at[pl.ds(r0, 8), pl.ds(c * 2048, 2048)],
                                      sem_wq.at[0]).start(priority=part)
    for s in range(LOOK):
        start_kv(s, s)

    prow = lax.broadcasted_iota(jnp.int32, (128, CHUNK), 0)
    pcol = lax.broadcasted_iota(jnp.int32, (128, CHUNK), 1)
    p_v[...] = jnp.where((pcol >> 5) == prow, 1.0, 0.0).astype(BF16)
    o_v[...] = jnp.zeros(o_v.shape, F32)
    outa_v[...] = jnp.zeros(outa_v.shape, F32)
    outb_v[...] = jnp.zeros(outb_v.shape, F32)
    qb_v[...] = jnp.zeros(qb_v.shape, F32)
    ctx_v[...] = jnp.zeros(ctx_v.shape, F32)
    wqb_v[pl.ds(DM * NH, N_WQB * CHUNK - DM * NH), :] = jnp.zeros(
        (N_WQB * CHUNK - DM * NH, DH), BF16)

    _wait(xb_v, sem_x.at[1])
    x8_v[...] = jnp.zeros(x8_v.shape, F32)
    x8_v[0:NB, 0:DM] = xb_v[...].astype(F32)
    for c in range(N_WQB):
        xbc_v[c] = x8_v[:, c * 128:(c + 1) * 128].astype(BF16)

    _wait(xa_v, sem_x.at[0])
    x8_v[0:NB, 0:DM] = xa_v[...].astype(F32)
    _wait(wq_v, sem_wq.at[0])
    qa = jnp.dot(x8_v[:, 0:DM].astype(BF16), wq_v[...], preferred_element_type=F32)
    for h in range(NH):
        q_v[h] = qa[:, h * DH:(h + 1) * DH].astype(BF16)

    def head_mask():
        r = lax.broadcasted_iota(jnp.int32, (128, CHUNK), 0)
        c = lax.broadcasted_iota(jnp.int32, (128, CHUNK), 1)
        return (r & 31) == (c & 31)

    nt = (((1,), (1,)), ((), ()))

    def step(i, carry):
        slot = i % KV_SLOTS
        h = i // NB
        b = i % NB

        @pl.when(i + LOOK < NSTEP)
        def _():
            start_kv(i + LOOK, (i + LOOK) % KV_SLOTS)

        def in_range(s0, n):
            return jnp.logical_and(i >= s0, i < s0 + n)

        def side_sem(step_issued):
            return sem_side.at[step_issued % N_SIDE_SEMS]

        @pl.when(in_range(S_WO, N_WO))
        def _():
            g = i - S_WO
            c0 = pl.multiple_of(g * WO_COLS, WO_COLS)
            ps = _pieces(DM, 24)
            half = len(ps) // 2
            for (r, n), prio in _interleave([(p_, 0) for p_ in ps[:half]], [(p_, 1) for p_ in ps[half:]]):
                pltpu.make_async_copy(wo_hbm.at[pl.ds(r, n), pl.ds(c0, WO_COLS)],
                                      wo_v.at[g, pl.ds(r, n)], sem_wo.at[g]).start(priority=prio)

        @pl.when(in_range(S_WQB, N_WQB - 1))
        def _():
            r0 = pl.multiple_of((i - S_WQB) * CHUNK, CHUNK)
            _start_rows(wqb_hbm, wqb_v, r0, r0, CHUNK, 224, side_sem(i))

        @pl.when(i == S_WQB + N_WQB - 1)
        def _():
            r0 = (N_WQB - 1) * CHUNK
            _start_rows(wqb_hbm, wqb_v, r0, r0, DM * NH - r0, 224, side_sem(i))

        @pl.when(in_range(S_WUK, N_WUK))
        def _():
            r0 = pl.multiple_of((i - S_WUK) * CHUNK, CHUNK)
            _start_rows(wuk_hbm, wuk_v, r0, r0, CHUNK, 224, side_sem(i))

        @pl.when(in_range(S_CKV, N_CKV))
        def _():
            n = i - S_CKV
            r0 = pl.multiple_of(n * CKV_ROWS, CKV_ROWS)
            _start_rows(ckv_hbm, ckv_v, r0, r0, CKV_ROWS, 48, side_sem(i))

        @pl.when(in_range(S_WUV, N_WUV))
        def _():
            r0 = pl.multiple_of((i - S_WUV) * CHUNK, CHUNK)
            _start_rows(wuv_hbm, wuv_v, r0, r0, CHUNK, 224, side_sem(i))

        @pl.when(in_range(S_WOB, N_WOB))
        def _():
            r0 = pl.multiple_of((i - S_WOB) * WOB_ROWS, WOB_ROWS)
            _start_rows(wob_hbm, wob_v, r0, r0, WOB_ROWS, 224, side_sem(i))

        _wait(kbuf.at[slot], sem_k.at[slot])
        s = lax.dot_general(q_v[h], kbuf[slot], nt, preferred_element_type=F32)
        m = jnp.max(s, axis=1, keepdims=True)
        p = jnp.exp((s - m) * SCALE)
        l = jnp.sum(p, axis=1, keepdims=True)
        _wait(vbuf.at[slot], sem_v.at[slot])
        o = jnp.dot(p.astype(BF16), vbuf[slot], preferred_element_type=F32) / l
        rows = lax.broadcasted_iota(jnp.int32, (8, DH), 0)
        o_v[h] = jnp.where(rows == b, o, o_v[h])

        @pl.when(jnp.logical_and(i % 32 == 31, i < NSTEP - 1))
        def _():
            g = i // 32
            _wait(wo_v.at[g], sem_wo.at[g])
            lhs = jnp.concatenate([o_v[g * 8 + hh] for hh in range(8)], axis=1).astype(BF16)
            outa_v[...] += lax.dot_general(lhs, wo_v[g], nt, preferred_element_type=F32)

        @pl.when(i == NSTEP - 2)
        def _():
            _wait(wo_v.at[3], sem_wo.at[3])
            lhs = jnp.concatenate([o_v[24 + hh] for hh in range(7)], axis=1).astype(BF16)
            outa_v[...] += lax.dot_general(lhs, wo_v[3, :, 0:7 * DH], nt,
                                           preferred_element_type=F32)

        j = i - LAG

        def job_range(s0, n):
            return jnp.logical_and(j >= s0, j < s0 + n)

        @pl.when(job_range(S_WQB, N_WQB - 1))
        def _():
            r0 = pl.multiple_of((j - S_WQB) * CHUNK, CHUNK)
            _wait(wqb_v.at[pl.ds(r0, CHUNK)], side_sem(j))

        @pl.when(j == S_WQB + N_WQB - 1)
        def _():
            r0 = (N_WQB - 1) * CHUNK
            _wait(wqb_v.at[pl.ds(r0, DM * NH - r0)], side_sem(j))

        @pl.when(job_range(S_WQB, N_WQB))
        def _():
            c = j - S_WQB
            r0 = pl.multiple_of(c * CHUNK, CHUNK)
            y = jnp.dot(xbc_v[c], p_v[...], preferred_element_type=F32)
            yb = jnp.broadcast_to(y[0:NB][:, None, :], (NB, NH, CHUNK)).reshape(128, CHUNK)
            x = jnp.where(head_mask(), yb, 0.0).astype(BF16)
            qb_v[...] += jnp.dot(x, wqb_v[pl.ds(r0, CHUNK), :], preferred_element_type=F32)

        @pl.when(job_range(S_WUK, N_WUK))
        def _():
            c = j - S_WUK
            r0 = pl.multiple_of(c * CHUNK, CHUNK)
            _wait(wuk_v.at[pl.ds(r0, CHUNK)], side_sem(j))
            g = lax.dot_general(qb_v[...].astype(BF16), wuk_v[pl.ds(r0, CHUNK), :], nt,
                                preferred_element_type=F32)
            gm = jnp.where(head_mask(), g, 0.0).astype(BF16)
            qabs_v[c] = lax.dot_general(gm, p_v[...], nt,
                                        preferred_element_type=F32).astype(BF16)

        @pl.when(job_range(S_CKV, N_CKV))
        def _():
            n = j - S_CKV
            bb = n // 4
            cc = n % 4
            r0 = pl.multiple_of(n * CKV_ROWS, CKV_ROWS)
            _wait(ckv_v.at[pl.ds(r0, CKV_ROWS)], side_sem(j))

            @pl.when(cc == 0)
            def _():
                m_v[...] = jnp.full(m_v.shape, -jnp.inf, F32)
                l_v[...] = jnp.zeros(l_v.shape, F32)
                acc_v[...] = jnp.zeros(acc_v.shape, F32)

            q0 = pl.multiple_of(bb * NH, NH)
            qq = jnp.concatenate([qabs_v[c, pl.ds(q0, NH), :] for c in range(4)], axis=1)
            kv = ckv_v[pl.ds(r0, CKV_ROWS), :]
            sb = lax.dot_general(qq, kv, nt, preferred_element_type=F32)
            m_old = m_v[...]
            m_new = jnp.maximum(m_old, jnp.max(sb, axis=1, keepdims=True))
            alpha = jnp.exp((m_old - m_new) * SCALE)
            pb = jnp.exp((sb - m_new) * SCALE)
            l_new = l_v[...] * alpha + jnp.sum(pb, axis=1, keepdims=True)
            acc = acc_v[...] * alpha + jnp.dot(pb.astype(BF16), kv, preferred_element_type=F32)
            m_v[...] = m_new
            l_v[...] = l_new
            acc_v[...] = acc

            @pl.when(cc == 3)
            def _():
                cl = (acc / l_new).astype(BF16)
                for c in range(4):
                    cl_v[c, pl.ds(q0, NH), :] = cl[:, c * 128:(c + 1) * 128]

        @pl.when(job_range(S_WUV, N_WUV))
        def _():
            c = j - S_WUV
            r0 = pl.multiple_of(c * CHUNK, CHUNK)
            _wait(wuv_v.at[pl.ds(r0, CHUNK)], side_sem(j))
            y = jnp.dot(cl_v[c], p_v[...], preferred_element_type=F32)
            e = jnp.where(head_mask(), y, 0.0).astype(BF16)
            ctx_v[...] += jnp.dot(e, wuv_v[pl.ds(r0, CHUNK), :], preferred_element_type=F32)

        @pl.when(job_range(S_WOB, N_WOB))
        def _():
            g = j - S_WOB
            r0 = pl.multiple_of(g * WOB_ROWS, WOB_ROWS)
            _wait(wob_v.at[pl.ds(r0, WOB_ROWS)], side_sem(j))

            @pl.when(g == 0)
            def _():
                r = lax.broadcasted_iota(jnp.int32, (NH * 8, 128), 0)
                c = lax.broadcasted_iota(jnp.int32, (NH * 8, 128), 1)
                perm = jnp.where(c == (r & 7) * NH + (r >> 3), 1.0, 0.0).astype(BF16)
                cp = jnp.dot(perm, ctx_v[...].astype(BF16), preferred_element_type=F32)
                for hh in range(NH):
                    cp_v[hh] = cp[hh * 8:(hh + 1) * 8].astype(BF16)

            acc = outb_v[...]
            for hh in range(8):
                rr = pl.multiple_of(r0 + hh * DM, 64)
                acc += lax.dot_general(cp_v[g * 8 + hh], wob_v[pl.ds(rr, DM), :], nt,
                                       preferred_element_type=F32)
            outb_v[...] = acc

        return carry

    lax.fori_loop(0, NSTEP, step, 0)

    outa = outa_v[...] + lax.dot_general(o_v[NH - 1].astype(BF16), wo_v[3, :, 7 * DH:8 * DH], nt,
                                         preferred_element_type=F32)
    res = jnp.concatenate([outa, outb_v[...]], axis=1)
    out_ref[...] = res[0:NB].astype(BF16)


@jax.jit
def pallas_concat_heads__mha_block_cached__compressed_kv_cla__decode_kernel(
    A_x: jax.Array,
    A_k_cache: jax.Array,
    A_v_cache: jax.Array,
    A_wq: jax.Array,
    A_wo: jax.Array,
    B_x: jax.Array,
    B_c_kv: jax.Array,
    B_w_q: jax.Array,
    B_w_uk: jax.Array,
    B_w_uv: jax.Array,
    B_w_o: jax.Array,
):
    ckv2 = B_c_kv.reshape(NB * SK, DC)
    wqb2 = B_w_q.reshape(DM * NH, DH)
    wuk2 = B_w_uk.reshape(DC * NH, DH)
    wuv2 = B_w_uv.reshape(DC * NH, DH)
    wob2 = B_w_o.transpose(0, 2, 1).reshape(NH * DM, DH)
    wo_t = A_wo.T
    xa2 = A_x.reshape(NB, DM)
    xb2 = B_x.reshape(NB, DM)

    vm = pltpu.VMEM
    scratch = [
        vm((NB, DM), BF16),
        vm((NB, DM), BF16),
        vm((KV_SLOTS, SK, DH), BF16),
        vm((KV_SLOTS, SK, DH), BF16),
        vm((DM, NH * DH), BF16),
        vm((N_WO, DM, WO_COLS), BF16),
        vm((N_WQB * CHUNK, DH), BF16),
        vm((DC * NH, DH), BF16),
        vm((DC * NH, DH), BF16),
        vm((NH * DM, DH), BF16),
        vm((NB * SK, DC), BF16),
        vm((128, CHUNK), BF16),
        vm((8, N_WQB * 128), F32),
        vm((N_WQB, 8, 128), BF16),
        vm((NH, 8, DH), BF16),
        vm((NH, 8, DH), F32),
        vm((128, DH), F32),
        vm((4, 128, 128), BF16),
        vm((NH, 1), F32),
        vm((NH, 1), F32),
        vm((NH, DC), F32),
        vm((4, 128, 128), BF16),
        vm((128, DH), F32),
        vm((NH, 8, DH), BF16),
        vm((8, DM), F32),
        vm((8, DM), F32),
        pltpu.SemaphoreType.DMA((2,)),
        pltpu.SemaphoreType.DMA((1,)),
        pltpu.SemaphoreType.DMA((KV_SLOTS,)),
        pltpu.SemaphoreType.DMA((KV_SLOTS,)),
        pltpu.SemaphoreType.DMA((N_WO,)),
        pltpu.SemaphoreType.DMA((N_SIDE_SEMS,)),
    ]
    out = pl.pallas_call(
        _kernel,
        out_shape=jax.ShapeDtypeStruct((NB, 2 * DM), BF16),
        in_specs=[pl.BlockSpec(memory_space=pl.ANY)] * 11,
        out_specs=pl.BlockSpec(memory_space=pltpu.VMEM),
        scratch_shapes=scratch,
        compiler_params=pltpu.CompilerParams(vmem_limit_bytes=110 * 1024 * 1024),
    )(xa2, A_k_cache, A_v_cache, A_wq, wo_t, xb2, ckv2, wqb2, wuk2, wuv2, wob2)
    return out.reshape(NB, 1, 2 * DM)
```

```python
import jax
import jax.numpy as jnp
from jax import lax
import jax.experimental.pallas as pl
import jax.experimental.pallas.tpu as pltpu

F32 = jnp.float32
BF16 = jnp.bfloat16

NB = 4
NH = 32
SK = 4096
DH = 128
DM = 576
DC = 512
SCALE = DH ** -0.5

HG = 8
NG = NH // HG
ROWS = 1024
NC = SK // ROWS
NIT = NG * NB * NC
PIECE = 128
NPIECE = ROWS // PIECE

CHUNK = 4096
CKV_ROWS = 1024
WOB_ROWS = 8 * DM
N_SIDE = 16

J_INIT = 1
J_B1, N_B1 = 18, 5
J_B2, N_B2 = J_B1 + N_B1, 4
J_B3, N_B3 = J_B2 + N_B2, 16
J_B4, N_B4 = J_B3 + N_B3, 4
J_B5, N_B5 = J_B4 + N_B4, 4

NT = (((1,), (1,)), ((), ()))


def _wait(buf_view, sem):
    pltpu.make_async_copy(buf_view, buf_view, sem).wait()


def _kernel(xa_hbm, k_hbm, v_hbm, wq_hbm, wo_hbm, xb_hbm, ckv_hbm, wqb_hbm, wuk_hbm, wuv_hbm,
            wob_hbm, out_ref,
            xa_v, xb_v, kbuf, vbuf, wq_v, wo_v, wqb_v, wuk_v, wuv_v, wob_v, ckv_v,
            p_v, x8_v, xbc_v, q8_v, ma_v, la_v, acca_v, o_v,
            qb_v, qabs_v, m_v, l_v, acc_v, cl_v, ctx_v, cp_v, outa_v, outb_v,
            sem_x, sem_wq, sem_k, sem_v, sem_vl, sem_side):

    def coords(it):
        return it // (NB * NC), (it // NC) % NB, it % NC

    def issue_kv(src, dst, sem, it, slot):
        g, b, c = coords(it)

        def body(r, carry):
            r0 = pl.multiple_of(r * PIECE, PIECE)
            s0 = pl.multiple_of(c * ROWS + r0, PIECE)
            for j in range(HG):
                pltpu.make_async_copy(src.at[b, g * HG + j, pl.ds(s0, PIECE)],
                                      dst.at[slot, j, pl.ds(r0, PIECE)],
                                      sem).start(priority=j % 2)
            return carry

        lax.fori_loop(0, NPIECE, body, 0)

    def issue_v_last(it, slot):
        g, b, c = coords(it)
        n = 0
        for j in range(HG):
            for r in range(NPIECE):
                pltpu.make_async_copy(v_hbm.at[b, g * HG + j, pl.ds(c * ROWS + r * PIECE, PIECE)],
                                      vbuf.at[slot, j, pl.ds(r * PIECE, PIECE)],
                                      sem_vl.at[j]).start(priority=n % 2)
                n += 1

    def issue_side(t):
        n = 0
        for p in range(9):
            if p < 8:
                for b in range(NB):
                    r0 = pl.multiple_of(b * SK + t * 256 + p * 32, 32)
                    pltpu.make_async_copy(ckv_hbm.at[pl.ds(r0, 32)], ckv_v.at[pl.ds(r0, 32)],
                                          sem_side.at[0]).start(priority=n % 2)
                    n += 1
            r9 = pl.multiple_of(t * (9 * PIECE) + p * PIECE, PIECE)
            pltpu.make_async_copy(wqb_hbm.at[pl.ds(r9, PIECE)], wqb_v.at[pl.ds(r9, PIECE)],
                                  sem_side.at[1]).start(priority=n % 2)
            n += 1
            if p < 8:
                r8 = pl.multiple_of(t * (8 * PIECE) + p * PIECE, PIECE)
                pltpu.make_async_copy(wuk_hbm.at[pl.ds(r8, PIECE)], wuk_v.at[pl.ds(r8, PIECE)],
                                      sem_side.at[2]).start(priority=n % 2)
                n += 1
                pltpu.make_async_copy(wuv_hbm.at[pl.ds(r8, PIECE)], wuv_v.at[pl.ds(r8, PIECE)],
                                      sem_side.at[3]).start(priority=n % 2)
                n += 1
            pltpu.make_async_copy(wob_hbm.at[pl.ds(r9, PIECE)], wob_v.at[pl.ds(r9, PIECE)],
                                  sem_side.at[4]).start(priority=n % 2)
            n += 1
            idx = t * 9 + p
            rr = pl.multiple_of((idx // 2) * 8, 8)
            cc = pl.multiple_of((idx % 2) * 2048, 2048)
            pltpu.make_async_copy(wo_hbm.at[pl.ds(rr, 8), pl.ds(cc, 2048)],
                                  wo_v.at[pl.ds(rr, 8), pl.ds(cc, 2048)],
                                  sem_side.at[5]).start(priority=n % 2)
            n += 1

    rows8 = lax.broadcasted_iota(jnp.int32, (8, DH), 0)

    def qk_softmax(it, slot):
        g, b, c = coords(it)
        q8 = q8_v[g * NB + b]
        s = None
        for j in range(HG):
            lhs = jnp.where(rows8 == j, q8, 0.0).astype(BF16)
            d = lax.dot_general(lhs, kbuf[slot, j], NT, preferred_element_type=F32)
            s = d if s is None else s + d
        first = c == 0
        m_old = jnp.where(first, -jnp.inf, ma_v[...])
        l_old = jnp.where(first, 0.0, la_v[...])
        m_new = jnp.maximum(m_old, jnp.max(s, axis=1, keepdims=True))
        alpha = jnp.exp((m_old - m_new) * SCALE)
        p = jnp.exp((s - m_new) * SCALE)
        l_new = l_old * alpha + jnp.sum(p, axis=1, keepdims=True)
        ma_v[...] = m_new
        la_v[...] = l_new
        return p.astype(BF16), alpha, l_new

    pltpu.make_async_copy(xa_hbm, xa_v, sem_x.at[0]).start()
    pltpu.make_async_copy(xb_hbm, xb_v, sem_x.at[1]).start()

    def wq_body(t, carry):
        for s in range(8):
            rr = pl.multiple_of((s * 9 + t // 2) * 8, 8)
            cc = pl.multiple_of((t % 2) * 2048, 2048)
            pltpu.make_async_copy(wq_hbm.at[pl.ds(rr, 8), pl.ds(cc, 2048)],
                                  wq_v.at[pl.ds(rr, 8), pl.ds(cc, 2048)],
                                  sem_wq.at[0]).start(priority=s % 2)
        return carry

    lax.fori_loop(0, 18, wq_body, 0)
    issue_kv(k_hbm, kbuf, sem_k.at[0], 0, 0)

    ma_v[...] = jnp.zeros(ma_v.shape, F32)
    la_v[...] = jnp.zeros(la_v.shape, F32)
    acca_v[...] = jnp.zeros(acca_v.shape, F32)
    o_v[...] = jnp.zeros(o_v.shape, F32)
    outa_v[...] = jnp.zeros(outa_v.shape, F32)
    x8_v[...] = jnp.zeros(x8_v.shape, F32)
    _wait(xa_v, sem_x.at[0])
    x8_v[0:NB, 0:DM] = xa_v[...].astype(F32)
    _wait(wq_v, sem_wq.at[0])
    qa = jnp.dot(x8_v[:, 0:DM].astype(BF16), wq_v[...], preferred_element_type=F32)
    qa = qa.astype(BF16).astype(F32)
    for g in range(NG):
        for b in range(NB):
            t = jnp.zeros((8, DH), F32)
            for j in range(HG):
                h = g * HG + j
                row = jnp.broadcast_to(qa[b:b + 1, h * DH:(h + 1) * DH], (8, DH))
                t = jnp.where(rows8 == j, row, t)
            q8_v[g * NB + b] = t

    issue_kv(v_hbm, vbuf, sem_v.at[0], 0, 0)

    def head_mask():
        r = lax.broadcasted_iota(jnp.int32, (128, CHUNK), 0)
        c = lax.broadcasted_iota(jnp.int32, (128, CHUNK), 1)
        return (r & 31) == (c & 31)

    def scatter_o(g, b, o):
        for j in range(HG):
            row = jnp.broadcast_to(o[j:j + 1, :], (8, DH))
            o_v[g * HG + j] = jnp.where(rows8 == b, row, o_v[g * HG + j])

    def project_group(g):
        lhs = jnp.concatenate([o_v[g * HG + j] for j in range(HG)], axis=1).astype(BF16)
        outa_v[...] += lax.dot_general(lhs, wo_v[:, g * HG * DH:(g + 1) * HG * DH], NT,
                                       preferred_element_type=F32)

    def step(i, carry):
        slot = i % 2
        g, b, c = coords(i)

        issue_kv(k_hbm, kbuf, sem_k.at[1 - slot], i + 1, 1 - slot)
        _wait(kbuf.at[slot], sem_k.at[slot])
        p, alpha, l_new = qk_softmax(i, slot)

        @pl.when(i + 1 < NIT - 1)
        def _():
            issue_kv(v_hbm, vbuf, sem_v.at[1 - slot], i + 1, 1 - slot)

        @pl.when(i + 1 == NIT - 1)
        def _():
            issue_v_last(NIT - 1, (NIT - 1) % 2)

        _wait(vbuf.at[slot], sem_v.at[slot])
        pv = None
        for j in range(HG):
            d = jnp.dot(p, vbuf[slot, j], preferred_element_type=F32)
            d = jnp.where(rows8 == j, d, 0.0)
            pv = d if pv is None else pv + d
        acc = jnp.where(c == 0, 0.0, acca_v[...] * alpha) + pv
        acca_v[...] = acc

        @pl.when(c == NC - 1)
        def _():
            scatter_o(g, b, acc / l_new)

        @pl.when(i < N_SIDE)
        def _():
            issue_side(i)

        for gg in range(NG - 1):
            @pl.when(i == (gg + 1) * NB * NC + 1)
            def _():
                if gg == 0:
                    _wait(wo_v, sem_side.at[5])
                project_group(gg)

        @pl.when(i == NIT - 2)
        def _():
            project_group(NG - 1)

        def job_range(s0, n):
            return jnp.logical_and(i >= s0, i < s0 + n)

        @pl.when(i == J_INIT)
        def _():
            prow = lax.broadcasted_iota(jnp.int32, (128, CHUNK), 0)
            pcol = lax.broadcasted_iota(jnp.int32, (128, CHUNK), 1)
            p_v[...] = jnp.where((pcol >> 5) == prow, 1.0, 0.0).astype(BF16)
            outb_v[...] = jnp.zeros(outb_v.shape, F32)
            qb_v[...] = jnp.zeros(qb_v.shape, F32)
            ctx_v[...] = jnp.zeros(ctx_v.shape, F32)
            wqb_v[pl.ds(DM * NH, N_B1 * CHUNK - DM * NH), :] = jnp.zeros(
                (N_B1 * CHUNK - DM * NH, DH), BF16)
            _wait(xb_v, sem_x.at[1])
            x8_v[0:NB, 0:DM] = xb_v[...].astype(F32)
            for cc in range(N_B1):
                xbc_v[cc] = x8_v[:, cc * 128:(cc + 1) * 128].astype(BF16)

        @pl.when(i == J_B1)
        def _():
            _wait(wqb_v.at[pl.ds(0, DM * NH)], sem_side.at[1])

        @pl.when(job_range(J_B1, N_B1))
        def _():
            cc = i - J_B1
            r0 = pl.multiple_of(cc * CHUNK, CHUNK)
            y = jnp.dot(xbc_v[cc], p_v[...], preferred_element_type=F32)
            yb = jnp.broadcast_to(y[0:NB][:, None, :], (NB, NH, CHUNK)).reshape(128, CHUNK)
            x = jnp.where(head_mask(), yb, 0.0).astype(BF16)
            qb_v[...] += jnp.dot(x, wqb_v[pl.ds(r0, CHUNK), :], preferred_element_type=F32)

        @pl.when(i == J_B2)
        def _():
            _wait(wuk_v, sem_side.at[2])

        @pl.when(job_range(J_B2, N_B2))
        def _():
            cc = i - J_B2
            r0 = pl.multiple_of(cc * CHUNK, CHUNK)
            gq = lax.dot_general(qb_v[...].astype(BF16), wuk_v[pl.ds(r0, CHUNK), :], NT,
                                 preferred_element_type=F32)
            gm = jnp.where(head_mask(), gq, 0.0).astype(BF16)
            qabs_v[cc] = lax.dot_general(gm, p_v[...], NT,
                                         preferred_element_type=F32).astype(BF16)

        @pl.when(i == J_B3)
        def _():
            _wait(ckv_v, sem_side.at[0])

        @pl.when(job_range(J_B3, N_B3))
        def _():
            n = i - J_B3
            bb = n // 4
            cc = n % 4
            r0 = pl.multiple_of(n * CKV_ROWS, CKV_ROWS)
            q0 = pl.multiple_of(bb * NH, NH)
            qq = jnp.concatenate([qabs_v[k, pl.ds(q0, NH), :] for k in range(4)], axis=1)
            kv = ckv_v[pl.ds(r0, CKV_ROWS), :]
            sb = lax.dot_general(qq, kv, NT, preferred_element_type=F32)

            @pl.when(cc == 0)
            def _():
                m_v[...] = jnp.full(m_v.shape, -jnp.inf, F32)
                l_v[...] = jnp.zeros(l_v.shape, F32)
                acc_v[...] = jnp.zeros(acc_v.shape, F32)

            m_old = m_v[...]
            m_new = jnp.maximum(m_old, jnp.max(sb, axis=1, keepdims=True))
            al = jnp.exp((m_old - m_new) * SCALE)
            pb = jnp.exp((sb - m_new) * SCALE)
            l_b = l_v[...] * al + jnp.sum(pb, axis=1, keepdims=True)
            accb = acc_v[...] * al + jnp.dot(pb.astype(BF16), kv, preferred_element_type=F32)
            m_v[...] = m_new
            l_v[...] = l_b
            acc_v[...] = accb

            @pl.when(cc == 3)
            def _():
                cl = (accb / l_b).astype(BF16)
                for k in range(4):
                    cl_v[k, pl.ds(q0, NH), :] = cl[:, k * 128:(k + 1) * 128]

        @pl.when(i == J_B4)
        def _():
            _wait(wuv_v, sem_side.at[3])

        @pl.when(job_range(J_B4, N_B4))
        def _():
            cc = i - J_B4
            r0 = pl.multiple_of(cc * CHUNK, CHUNK)
            y = jnp.dot(cl_v[cc], p_v[...], preferred_element_type=F32)
            e = jnp.where(head_mask(), y, 0.0).astype(BF16)
            ctx_v[...] += jnp.dot(e, wuv_v[pl.ds(r0, CHUNK), :], preferred_element_type=F32)

        @pl.when(i == J_B5)
        def _():
            _wait(wob_v, sem_side.at[4])
            r = lax.broadcasted_iota(jnp.int32, (NH * 8, 128), 0)
            cc = lax.broadcasted_iota(jnp.int32, (NH * 8, 128), 1)
            valid = (r & 7) < NB
            perm = jnp.where(jnp.logical_and(valid, cc == (r & 7) * NH + (r >> 3)), 1.0, 0.0)
            cp = jnp.dot(perm.astype(BF16), ctx_v[...].astype(BF16), preferred_element_type=F32)
            for hh in range(NH):
                cp_v[hh] = cp[hh * 8:(hh + 1) * 8].astype(BF16)

        @pl.when(job_range(J_B5, N_B5))
        def _():
            gb = i - J_B5
            r0 = pl.multiple_of(gb * WOB_ROWS, WOB_ROWS)
            accb = outb_v[...]
            for hh in range(8):
                rr = pl.multiple_of(r0 + hh * DM, 64)
                accb += lax.dot_general(cp_v[gb * 8 + hh], wob_v[pl.ds(rr, DM), :], NT,
                                        preferred_element_type=F32)
            outb_v[...] = accb

        return carry

    lax.fori_loop(0, NIT - 1, step, 0)

    it = NIT - 1
    slot = it % 2
    g = NG - 1
    _wait(kbuf.at[slot], sem_k.at[slot])
    p, alpha, l_new = qk_softmax(it, slot)
    inv_l = 1.0 / l_new
    base = acca_v[...] * alpha
    last = jnp.zeros((8, DM), F32)
    for j in range(HG):
        _wait(vbuf.at[slot, j], sem_vl.at[j])
        o = (base + jnp.dot(p, vbuf[slot, j], preferred_element_type=F32)) * inv_l
        h = g * HG + j
        d = lax.dot_general(o.astype(BF16), wo_v[:, h * DH:(h + 1) * DH], NT,
                            preferred_element_type=F32)
        last = last + jnp.where(lax.broadcasted_iota(jnp.int32, (8, DM), 0) == j, d, 0.0)
    last_row = jnp.sum(last, axis=0, keepdims=True)
    rows_m = lax.broadcasted_iota(jnp.int32, (8, DM), 0)
    outa = outa_v[...] + jnp.where(rows_m == NB - 1, jnp.broadcast_to(last_row, (8, DM)), 0.0)
    res = jnp.concatenate([outa, outb_v[...]], axis=1)
    out_ref[...] = res[0:NB].astype(BF16)


@jax.jit
def pallas_concat_heads__mha_block_cached__compressed_kv_cla__decode_kernel(
    A_x: jax.Array,
    A_k_cache: jax.Array,
    A_v_cache: jax.Array,
    A_wq: jax.Array,
    A_wo: jax.Array,
    B_x: jax.Array,
    B_c_kv: jax.Array,
    B_w_q: jax.Array,
    B_w_uk: jax.Array,
    B_w_uv: jax.Array,
    B_w_o: jax.Array,
):
    ckv2 = B_c_kv.reshape(NB * SK, DC)
    wqb2 = B_w_q.reshape(DM * NH, DH)
    wuk2 = B_w_uk.reshape(DC * NH, DH)
    wuv2 = B_w_uv.reshape(DC * NH, DH)
    wob2 = B_w_o.transpose(0, 2, 1).reshape(NH * DM, DH)
    wo_t = A_wo.T
    xa2 = A_x.reshape(NB, DM)
    xb2 = B_x.reshape(NB, DM)

    vm = pltpu.VMEM
    n_b1_rows = N_B1 * CHUNK
    scratch = [
        vm((NB, DM), BF16),
        vm((NB, DM), BF16),
        vm((2, HG, ROWS, DH), BF16),
        vm((2, HG, ROWS, DH), BF16),
        vm((DM, NH * DH), BF16),
        vm((DM, NH * DH), BF16),
        vm((n_b1_rows, DH), BF16),
        vm((DC * NH, DH), BF16),
        vm((DC * NH, DH), BF16),
        vm((NH * DM, DH), BF16),
        vm((NB * SK, DC), BF16),
        vm((128, CHUNK), BF16),
        vm((8, N_B1 * 128), F32),
        vm((N_B1, 8, 128), BF16),
        vm((NG * NB, 8, DH), F32),
        vm((8, 1), F32),
        vm((8, 1), F32),
        vm((8, DH), F32),
        vm((NH, 8, DH), F32),
        vm((128, DH), F32),
        vm((4, 128, 128), BF16),
        vm((NH, 1), F32),
        vm((NH, 1), F32),
        vm((NH, DC), F32),
        vm((4, 128, 128), BF16),
        vm((128, DH), F32),
        vm((NH, 8, DH), BF16),
        vm((8, DM), F32),
        vm((8, DM), F32),
        pltpu.SemaphoreType.DMA((2,)),
        pltpu.SemaphoreType.DMA((1,)),
        pltpu.SemaphoreType.DMA((2,)),
        pltpu.SemaphoreType.DMA((2,)),
        pltpu.SemaphoreType.DMA((HG,)),
        pltpu.SemaphoreType.DMA((6,)),
    ]
    out = pl.pallas_call(
        _kernel,
        out_shape=jax.ShapeDtypeStruct((NB, 2 * DM), BF16),
        in_specs=[pl.BlockSpec(memory_space=pl.ANY)] * 11,
        out_specs=pl.BlockSpec(memory_space=pltpu.VMEM),
        scratch_shapes=scratch,
        compiler_params=pltpu.CompilerParams(vmem_limit_bytes=110 * 1024 * 1024),
    )(xa2, A_k_cache, A_v_cache, A_wq, wo_t, xb2, ckv2, wqb2, wuk2, wuv2, wob2)
    return out.reshape(NB, 1, 2 * DM)
```

```python
import jax
import jax.numpy as jnp
from jax import lax
import jax.experimental.pallas as pl
import jax.experimental.pallas.tpu as pltpu

F32 = jnp.float32
BF16 = jnp.bfloat16

NB = 4
NH = 32
SK = 4096
DH = 128
DM = 576
DC = 512
SCALE = DH ** -0.5

HG = 8
NG = NH // HG
ROWS = 1024
NC = SK // ROWS
NIT = NG * NB * NC
PIECE = 128
NPIECE = ROWS // PIECE

CHUNK = 4096
CKV_ROWS = 1024
WOB_ROWS = 8 * DM

J_INIT = 1
J_B1, N_B1 = 18, 5
J_B2, N_B2 = J_B1 + N_B1, 4
J_B3, N_B3 = J_B2 + N_B2, 16
J_B4, N_B4 = J_B3 + N_B3, 4
J_B5, N_B5 = J_B4 + N_B4, 4

NT = (((1,), (1,)), ((), ()))

LAST_Q0 = (0, 1, 2)
LAST_Q1 = (4, 5, 6)
LAST_SHARED = (7, 3)
LAST_BLOCKS = ((0, 4), (1, 5), (2, 6), (7,), (3,))


def _wait(buf_view, sem):
    pltpu.make_async_copy(buf_view, buf_view, sem).wait()


def _kernel(xa_hbm, k_hbm, v_hbm, wq_hbm, wo_hbm, xb_hbm, ckv_hbm, wqb_hbm, wuk_hbm, wuv_hbm,
            wob_hbm, out_ref,
            xa_v, xb_v, kbuf, vbuf, wq_v, wo_v, wqb_v, wuk_v, wuv_v, wob_v, ckv_v,
            p_v, x8_v, xbc_v, q8_v, ma_v, la_v, pa_v, al_v, ll_v, acca_v, o_v,
            qb_v, qabs_v, m_v, l_v, acc_v, cl_v, ctx_v, cp_v, outa_v, outb_v,
            sem_x, sem_wq, sem_k, sem_v, sem_vl, sem_side):

    def coords(it):
        return it // (NB * NC), (it // NC) % NB, it % NC

    def issue_kv(src, dst, sem, it, slot):
        g, b, c = coords(it)

        def body(r, carry):
            r0 = pl.multiple_of(r * PIECE, PIECE)
            s0 = pl.multiple_of(c * ROWS + r0, PIECE)
            for j in range(HG):
                pltpu.make_async_copy(src.at[b, g * HG + j, pl.ds(s0, PIECE)],
                                      dst.at[slot, j, pl.ds(r0, PIECE)],
                                      sem).start(priority=j % 2)
            return carry

        lax.fori_loop(0, NPIECE, body, 0)

    def issue_v_last(it, slot):
        g, b, c = coords(it)
        q0 = [(j, r) for j in LAST_Q0 for r in range(NPIECE)]
        q1 = [(j, r) for j in LAST_Q1 for r in range(NPIECE)]
        for j in LAST_SHARED:
            q0 += [(j, r) for r in range(0, NPIECE, 2)]
            q1 += [(j, r) for r in range(1, NPIECE, 2)]
        for pair in zip(q0, q1):
            for prio, (j, r) in enumerate(pair):
                pltpu.make_async_copy(v_hbm.at[b, g * HG + j, pl.ds(c * ROWS + r * PIECE, PIECE)],
                                      vbuf.at[slot, j, pl.ds(r * PIECE, PIECE)],
                                      sem_vl.at[j]).start(priority=prio)

    def issue_wide(src, dst, sem, t0, t1):
        def body(t, carry):
            for s in range(8):
                rr = pl.multiple_of((s * 9 + t // 2) * 8, 8)
                cc = pl.multiple_of((t % 2) * 2048, 2048)
                pltpu.make_async_copy(src.at[pl.ds(rr, 8), pl.ds(cc, 2048)],
                                      dst.at[pl.ds(rr, 8), pl.ds(cc, 2048)],
                                      sem).start(priority=s % 2)
            return carry

        lax.fori_loop(t0, t1, body, 0)

    def issue_ckv(t):
        def body(p, carry):
            for s in range(8):
                r0 = pl.multiple_of(s * 2048 + t * 256 + p * 32, 32)
                pltpu.make_async_copy(ckv_hbm.at[pl.ds(r0, 32)], ckv_v.at[pl.ds(r0, 32)],
                                      sem_side.at[0]).start(priority=s % 2)
            return carry

        lax.fori_loop(0, 8, body, 0)

    def issue_weights(t):
        def pair(p, with_small):
            for half in range(2):
                r9 = pl.multiple_of(half * (72 * PIECE) + (t * 9 + p) * PIECE, PIECE)
                pltpu.make_async_copy(wqb_hbm.at[pl.ds(r9, PIECE)], wqb_v.at[pl.ds(r9, PIECE)],
                                      sem_side.at[1]).start(priority=0)
                pltpu.make_async_copy(wob_hbm.at[pl.ds(r9, PIECE)], wob_v.at[pl.ds(r9, PIECE)],
                                      sem_side.at[4]).start(priority=1)
                if with_small:
                    r8 = pl.multiple_of(half * (64 * PIECE) + (t * 8 + p) * PIECE, PIECE)
                    pltpu.make_async_copy(wuk_hbm.at[pl.ds(r8, PIECE)],
                                          wuk_v.at[pl.ds(r8, PIECE)],
                                          sem_side.at[2]).start(priority=0)
                    pltpu.make_async_copy(wuv_hbm.at[pl.ds(r8, PIECE)],
                                          wuv_v.at[pl.ds(r8, PIECE)],
                                          sem_side.at[3]).start(priority=1)

        def body(p, carry):
            pair(p, True)
            return carry

        lax.fori_loop(0, 8, body, 0)
        pair(8, False)

    rows8 = lax.broadcasted_iota(jnp.int32, (8, DH), 0)

    def qk_softmax(it):
        slot = it % 2
        g, b, c = coords(it)
        q8 = q8_v[g * NB + b]
        s = None
        for j in range(HG):
            lhs = jnp.where(rows8 == j, q8, 0.0).astype(BF16)
            d = lax.dot_general(lhs, kbuf[slot, j], NT, preferred_element_type=F32)
            s = d if s is None else s + d
        first = c == 0
        m_old = jnp.where(first, -jnp.inf, ma_v[...])
        l_old = jnp.where(first, 0.0, la_v[...])
        m_new = jnp.maximum(m_old, jnp.max(s, axis=1, keepdims=True))
        alpha = jnp.exp((m_old - m_new) * SCALE)
        p = jnp.exp((s - m_new) * SCALE)
        l_new = l_old * alpha + jnp.sum(p, axis=1, keepdims=True)
        ma_v[...] = m_new
        la_v[...] = l_new
        pa_v[slot] = p.astype(BF16)
        al_v[slot] = alpha
        ll_v[slot] = l_new

    pltpu.make_async_copy(xa_hbm, xa_v, sem_x.at[0]).start()
    pltpu.make_async_copy(xb_hbm, xb_v, sem_x.at[1]).start()

    issue_wide(wq_hbm, wq_v, sem_wq.at[0], 0, 18)
    issue_kv(k_hbm, kbuf, sem_k.at[0], 0, 0)

    ma_v[...] = jnp.zeros(ma_v.shape, F32)
    la_v[...] = jnp.zeros(la_v.shape, F32)
    acca_v[...] = jnp.zeros(acca_v.shape, F32)
    o_v[...] = jnp.zeros(o_v.shape, F32)
    outa_v[...] = jnp.zeros(outa_v.shape, F32)
    x8_v[...] = jnp.zeros(x8_v.shape, F32)
    _wait(xa_v, sem_x.at[0])
    x8_v[0:NB, 0:DM] = xa_v[...].astype(F32)
    _wait(wq_v, sem_wq.at[0])
    qa = jnp.dot(x8_v[:, 0:DM].astype(BF16), wq_v[...], preferred_element_type=F32)
    qa = qa.astype(BF16).astype(F32)
    for g in range(NG):
        for b in range(NB):
            t = jnp.zeros((8, DH), F32)
            for j in range(HG):
                h = g * HG + j
                row = jnp.broadcast_to(qa[b:b + 1, h * DH:(h + 1) * DH], (8, DH))
                t = jnp.where(rows8 == j, row, t)
            q8_v[g * NB + b] = t

    def head_mask():
        r = lax.broadcasted_iota(jnp.int32, (128, CHUNK), 0)
        c = lax.broadcasted_iota(jnp.int32, (128, CHUNK), 1)
        return (r & 31) == (c & 31)

    def scatter_o(g, b, o):
        for j in range(HG):
            row = jnp.broadcast_to(o[j:j + 1, :], (8, DH))
            o_v[g * HG + j] = jnp.where(rows8 == b, row, o_v[g * HG + j])

    def project_group(g):
        lhs = jnp.concatenate([o_v[g * HG + j] for j in range(HG)], axis=1).astype(BF16)
        outa_v[...] += lax.dot_general(lhs, wo_v[:, g * HG * DH:(g + 1) * HG * DH], NT,
                                       preferred_element_type=F32)

    def step(i, carry):
        slot = (i + 2) % 2
        nxt = 1 - slot

        @pl.when(i + 2 < NIT)
        def _():
            issue_kv(k_hbm, kbuf, sem_k.at[slot], i + 2, slot)

        _wait(kbuf.at[nxt], sem_k.at[nxt])
        qk_softmax(i + 1)

        @pl.when(i + 1 < NIT - 1)
        def _():
            issue_kv(v_hbm, vbuf, sem_v.at[nxt], i + 1, nxt)

        @pl.when(i + 1 == NIT - 1)
        def _():
            issue_v_last(NIT - 1, (NIT - 1) % 2)

        @pl.when(i >= 0)
        def _():
            g, b, c = coords(i)
            _wait(vbuf.at[slot], sem_v.at[slot])
            p = pa_v[slot]
            pv = None
            for j in range(HG):
                d = jnp.dot(p, vbuf[slot, j], preferred_element_type=F32)
                d = jnp.where(rows8 == j, d, 0.0)
                pv = d if pv is None else pv + d
            acc = jnp.where(c == 0, 0.0, acca_v[...] * al_v[slot]) + pv
            acca_v[...] = acc

            @pl.when(c == NC - 1)
            def _():
                scatter_o(g, b, acc / ll_v[slot])

        @pl.when(jnp.logical_and(i >= 0, i < 8))
        def _():
            issue_ckv(i)

        @pl.when(jnp.logical_and(i >= 8, i < 16))
        def _():
            issue_weights(i - 8)

        @pl.when(jnp.logical_and(i >= 16, i < 18))
        def _():
            issue_wide(wo_hbm, wo_v, sem_side.at[5], (i - 16) * 9, (i - 15) * 9)

        for gg in range(NG - 1):
            @pl.when(i == (gg + 1) * NB * NC + 5)
            def _():
                if gg == 0:
                    _wait(wo_v, sem_side.at[5])
                project_group(gg)

        @pl.when(i == NIT - NC)
        def _():
            project_group(NG - 1)

        def job_range(s0, n):
            return jnp.logical_and(i >= s0, i < s0 + n)

        @pl.when(i == J_INIT)
        def _():
            prow = lax.broadcasted_iota(jnp.int32, (128, CHUNK), 0)
            pcol = lax.broadcasted_iota(jnp.int32, (128, CHUNK), 1)
            p_v[...] = jnp.where((pcol >> 5) == prow, 1.0, 0.0).astype(BF16)
            outb_v[...] = jnp.zeros(outb_v.shape, F32)
            qb_v[...] = jnp.zeros(qb_v.shape, F32)
            ctx_v[...] = jnp.zeros(ctx_v.shape, F32)
            wqb_v[pl.ds(DM * NH, N_B1 * CHUNK - DM * NH), :] = jnp.zeros(
                (N_B1 * CHUNK - DM * NH, DH), BF16)
            _wait(xb_v, sem_x.at[1])
            x8_v[0:NB, 0:DM] = xb_v[...].astype(F32)
            for cc in range(N_B1):
                xbc_v[cc] = x8_v[:, cc * 128:(cc + 1) * 128].astype(BF16)

        @pl.when(i == J_B1)
        def _():
            _wait(wqb_v.at[pl.ds(0, DM * NH)], sem_side.at[1])

        @pl.when(job_range(J_B1, N_B1))
        def _():
            cc = i - J_B1
            r0 = pl.multiple_of(cc * CHUNK, CHUNK)
            y = jnp.dot(xbc_v[cc], p_v[...], preferred_element_type=F32)
            yb = jnp.broadcast_to(y[0:NB][:, None, :], (NB, NH, CHUNK)).reshape(128, CHUNK)
            x = jnp.where(head_mask(), yb, 0.0).astype(BF16)
            qb_v[...] += jnp.dot(x, wqb_v[pl.ds(r0, CHUNK), :], preferred_element_type=F32)

        @pl.when(i == J_B2)
        def _():
            _wait(wuk_v, sem_side.at[2])

        @pl.when(job_range(J_B2, N_B2))
        def _():
            cc = i - J_B2
            r0 = pl.multiple_of(cc * CHUNK, CHUNK)
            gq = lax.dot_general(qb_v[...].astype(BF16), wuk_v[pl.ds(r0, CHUNK), :], NT,
                                 preferred_element_type=F32)
            gm = jnp.where(head_mask(), gq, 0.0).astype(BF16)
            qabs_v[cc] = lax.dot_general(gm, p_v[...], NT,
                                         preferred_element_type=F32).astype(BF16)

        @pl.when(i == J_B3)
        def _():
            _wait(ckv_v, sem_side.at[0])

        @pl.when(job_range(J_B3, N_B3))
        def _():
            n = i - J_B3
            bb = n // 4
            cc = n % 4
            r0 = pl.multiple_of(n * CKV_ROWS, CKV_ROWS)
            q0 = pl.multiple_of(bb * NH, NH)
            qq = jnp.concatenate([qabs_v[k, pl.ds(q0, NH), :] for k in range(4)], axis=1)
            kv = ckv_v[pl.ds(r0, CKV_ROWS), :]
            sb = lax.dot_general(qq, kv, NT, preferred_element_type=F32)

            @pl.when(cc == 0)
            def _():
                m_v[...] = jnp.full(m_v.shape, -jnp.inf, F32)
                l_v[...] = jnp.zeros(l_v.shape, F32)
                acc_v[...] = jnp.zeros(acc_v.shape, F32)

            m_old = m_v[...]
            m_new = jnp.maximum(m_old, jnp.max(sb, axis=1, keepdims=True))
            al = jnp.exp((m_old - m_new) * SCALE)
            pb = jnp.exp((sb - m_new) * SCALE)
            l_b = l_v[...] * al + jnp.sum(pb, axis=1, keepdims=True)
            accb = acc_v[...] * al + jnp.dot(pb.astype(BF16), kv, preferred_element_type=F32)
            m_v[...] = m_new
            l_v[...] = l_b
            acc_v[...] = accb

            @pl.when(cc == 3)
            def _():
                cl = (accb / l_b).astype(BF16)
                for k in range(4):
                    cl_v[k, pl.ds(q0, NH), :] = cl[:, k * 128:(k + 1) * 128]

        @pl.when(i == J_B4)
        def _():
            _wait(wuv_v, sem_side.at[3])

        @pl.when(job_range(J_B4, N_B4))
        def _():
            cc = i - J_B4
            r0 = pl.multiple_of(cc * CHUNK, CHUNK)
            y = jnp.dot(cl_v[cc], p_v[...], preferred_element_type=F32)
            e = jnp.where(head_mask(), y, 0.0).astype(BF16)
            ctx_v[...] += jnp.dot(e, wuv_v[pl.ds(r0, CHUNK), :], preferred_element_type=F32)

        @pl.when(i == J_B5)
        def _():
            _wait(wob_v, sem_side.at[4])
            r = lax.broadcasted_iota(jnp.int32, (NH * 8, 128), 0)
            cc = lax.broadcasted_iota(jnp.int32, (NH * 8, 128), 1)
            valid = (r & 7) < NB
            perm = jnp.where(jnp.logical_and(valid, cc == (r & 7) * NH + (r >> 3)), 1.0, 0.0)
            cp = jnp.dot(perm.astype(BF16), ctx_v[...].astype(BF16), preferred_element_type=F32)
            for hh in range(NH):
                cp_v[hh] = cp[hh * 8:(hh + 1) * 8].astype(BF16)

        @pl.when(job_range(J_B5, N_B5))
        def _():
            gb = i - J_B5
            r0 = pl.multiple_of(gb * WOB_ROWS, WOB_ROWS)
            accb = outb_v[...]
            for hh in range(8):
                rr = pl.multiple_of(r0 + hh * DM, 64)
                accb += lax.dot_general(cp_v[gb * 8 + hh], wob_v[pl.ds(rr, DM), :], NT,
                                        preferred_element_type=F32)
            outb_v[...] = accb

        return carry

    lax.fori_loop(-1, NIT - 1, step, 0)

    it = NIT - 1
    slot = it % 2
    g = NG - 1
    p = pa_v[slot]
    inv_l = 1.0 / ll_v[slot]
    base = acca_v[...] * al_v[slot]
    rows_m = lax.broadcasted_iota(jnp.int32, (8, DM), 0)

    def last_heads(js):
        for j in js:
            _wait(vbuf.at[slot, j], sem_vl.at[j])
        res = None
        for j in js:
            o = (base + jnp.dot(p, vbuf[slot, j], preferred_element_type=F32)) * inv_l
            h = g * HG + j
            d = lax.dot_general(o.astype(BF16), wo_v[:, h * DH:(h + 1) * DH], NT,
                                preferred_element_type=F32)
            d = jnp.where(rows_m == j, d, 0.0)
            res = d if res is None else res + d
        return res

    part = None
    for js in LAST_BLOCKS[:-1]:
        d = last_heads(js)
        part = d if part is None else part + d
    part_row = jnp.broadcast_to(jnp.sum(part, axis=0, keepdims=True), (8, DM))
    outa = outa_v[...] + jnp.where(rows_m == NB - 1, part_row, 0.0)
    outa = outa + last_heads(LAST_BLOCKS[-1])
    res = jnp.concatenate([outa, outb_v[...]], axis=1)
    out_ref[...] = res[0:NB].astype(BF16)


@jax.jit
def pallas_concat_heads__mha_block_cached__compressed_kv_cla__decode_kernel(
    A_x: jax.Array,
    A_k_cache: jax.Array,
    A_v_cache: jax.Array,
    A_wq: jax.Array,
    A_wo: jax.Array,
    B_x: jax.Array,
    B_c_kv: jax.Array,
    B_w_q: jax.Array,
    B_w_uk: jax.Array,
    B_w_uv: jax.Array,
    B_w_o: jax.Array,
):
    ckv2 = B_c_kv.reshape(NB * SK, DC)
    wqb2 = B_w_q.reshape(DM * NH, DH)
    wuk2 = B_w_uk.reshape(DC * NH, DH)
    wuv2 = B_w_uv.reshape(DC * NH, DH)
    wob2 = B_w_o.transpose(0, 2, 1).reshape(NH * DM, DH)
    wo_t = A_wo.T
    xa2 = A_x.reshape(NB, DM)
    xb2 = B_x.reshape(NB, DM)

    vm = pltpu.VMEM
    n_b1_rows = N_B1 * CHUNK
    scratch = [
        vm((NB, DM), BF16),
        vm((NB, DM), BF16),
        vm((2, HG, ROWS, DH), BF16),
        vm((2, HG, ROWS, DH), BF16),
        vm((DM, NH * DH), BF16),
        vm((DM, NH * DH), BF16),
        vm((n_b1_rows, DH), BF16),
        vm((DC * NH, DH), BF16),
        vm((DC * NH, DH), BF16),
        vm((NH * DM, DH), BF16),
        vm((NB * SK, DC), BF16),
        vm((128, CHUNK), BF16),
        vm((8, N_B1 * 128), F32),
        vm((N_B1, 8, 128), BF16),
        vm((NG * NB, 8, DH), F32),
        vm((8, 1), F32),
        vm((8, 1), F32),
        vm((2, 8, ROWS), BF16),
        vm((2, 8, 1), F32),
        vm((2, 8, 1), F32),
        vm((8, DH), F32),
        vm((NH, 8, DH), F32),
        vm((128, DH), F32),
        vm((4, 128, 128), BF16),
        vm((NH, 1), F32),
        vm((NH, 1), F32),
        vm((NH, DC), F32),
        vm((4, 128, 128), BF16),
        vm((128, DH), F32),
        vm((NH, 8, DH), BF16),
        vm((8, DM), F32),
        vm((8, DM), F32),
        pltpu.SemaphoreType.DMA((2,)),
        pltpu.SemaphoreType.DMA((1,)),
        pltpu.SemaphoreType.DMA((2,)),
        pltpu.SemaphoreType.DMA((2,)),
        pltpu.SemaphoreType.DMA((HG,)),
        pltpu.SemaphoreType.DMA((6,)),
    ]
    out = pl.pallas_call(
        _kernel,
        out_shape=jax.ShapeDtypeStruct((NB, 2 * DM), BF16),
        in_specs=[pl.BlockSpec(memory_space=pl.ANY)] * 11,
        out_specs=pl.BlockSpec(memory_space=pltpu.VMEM),
        scratch_shapes=scratch,
        compiler_params=pltpu.CompilerParams(vmem_limit_bytes=110 * 1024 * 1024,
                                             disable_semaphore_checks=True),
    )(xa2, A_k_cache, A_v_cache, A_wq, wo_t, xb2, ckv2, wqb2, wuk2, wuv2, wob2)
    return out.reshape(NB, 1, 2 * DM)
```

```python
import jax
import jax.numpy as jnp
from jax import lax
import jax.experimental.pallas as pl
import jax.experimental.pallas.tpu as pltpu

F32 = jnp.float32
BF16 = jnp.bfloat16

NB = 4
NH = 32
SK = 4096
DH = 128
DM = 576
DC = 512
SCALE = DH ** -0.5

HG = 8
NG = NH // HG
ROWS = 1024
NC = SK // ROWS
NIT = NG * NB * NC
PIECE = 128
NPIECE = ROWS // PIECE

CHUNK = 4096
CKV_ROWS = 1024
WOB_ROWS = 8 * DM

J_INIT = 1
J_B1, N_B1 = 18, 5
J_B2, N_B2 = J_B1 + N_B1, 4
J_B3, N_B3 = J_B2 + N_B2, 16
J_B4, N_B4 = J_B3 + N_B3, 4
J_B5, N_B5 = J_B4 + N_B4, 4

NT = (((1,), (1,)), ((), ()))

LAST_Q0 = (0, 2, 4, 6)
LAST_Q1 = (1, 5, 7, 3)


def _wait(buf_view, sem):
    pltpu.make_async_copy(buf_view, buf_view, sem).wait()


def _kernel(xa_hbm, k_hbm, v_hbm, wq_hbm, wo_hbm, xb_hbm, ckv_hbm, wqb_hbm, wuk_hbm, wuv_hbm,
            wob_hbm, out_ref,
            xa_v, xb_v, kbuf, vbuf, wq_v, wo_v, wqb_v, wuk_v, wuv_v, wob_v, ckv_v,
            p_v, x8_v, xbc_v, q8_v, ma_v, la_v, pa_v, al_v, ll_v, acca_v, o_v,
            qb_v, qabs_v, m_v, l_v, acc_v, cl_v, ctx_v, cp_v, outa_v, outb_v,
            sem_x, sem_wq, sem_k, sem_v, sem_vp, sem_vl, sem_side):

    def coords(it):
        return it // (NB * NC), (it // NC) % NB, it % NC

    def issue_kv(src, dst, sems, it, slot):
        g, b, c = coords(it)

        def body(r, carry):
            r0 = pl.multiple_of(r * PIECE, PIECE)
            s0 = pl.multiple_of(c * ROWS + r0, PIECE)
            for j in range(HG):
                pltpu.make_async_copy(src.at[b, g * HG + j, pl.ds(s0, PIECE)],
                                      dst.at[slot, j, pl.ds(r0, PIECE)],
                                      sems[j % 2]).start(priority=j % 2)
            return carry

        lax.fori_loop(0, NPIECE, body, 0)

    def issue_v_last(it, slot):
        g, b, c = coords(it)
        q0 = [(j, r) for j in LAST_Q0 for r in range(NPIECE)]
        q1 = [(j, r) for j in LAST_Q1 for r in range(NPIECE)]
        for pair in zip(q0, q1):
            for prio, (j, r) in enumerate(pair):
                pltpu.make_async_copy(v_hbm.at[b, g * HG + j, pl.ds(c * ROWS + r * PIECE, PIECE)],
                                      vbuf.at[slot, j, pl.ds(r * PIECE, PIECE)],
                                      sem_vl.at[j]).start(priority=prio)

    def issue_wide(src, dst, sem, t0, t1):
        def body(t, carry):
            for s in range(8):
                rr = pl.multiple_of((s * 9 + t // 2) * 8, 8)
                cc = pl.multiple_of((t % 2) * 2048, 2048)
                pltpu.make_async_copy(src.at[pl.ds(rr, 8), pl.ds(cc, 2048)],
                                      dst.at[pl.ds(rr, 8), pl.ds(cc, 2048)],
                                      sem).start(priority=s % 2)
            return carry

        lax.fori_loop(t0, t1, body, 0)

    def issue_ckv(t):
        def body(p, carry):
            for s in range(8):
                r0 = pl.multiple_of(s * 2048 + t * 256 + p * 32, 32)
                pltpu.make_async_copy(ckv_hbm.at[pl.ds(r0, 32)], ckv_v.at[pl.ds(r0, 32)],
                                      sem_side.at[0]).start(priority=s % 2)
            return carry

        lax.fori_loop(0, 8, body, 0)

    def issue_weights(t):
        def pair(p, with_small):
            for half in range(2):
                r9 = pl.multiple_of(half * (72 * PIECE) + (t * 9 + p) * PIECE, PIECE)
                pltpu.make_async_copy(wqb_hbm.at[pl.ds(r9, PIECE)], wqb_v.at[pl.ds(r9, PIECE)],
                                      sem_side.at[1]).start(priority=0)
                pltpu.make_async_copy(wob_hbm.at[pl.ds(r9, PIECE)], wob_v.at[pl.ds(r9, PIECE)],
                                      sem_side.at[4]).start(priority=1)
                if with_small:
                    r8 = pl.multiple_of(half * (64 * PIECE) + (t * 8 + p) * PIECE, PIECE)
                    pltpu.make_async_copy(wuk_hbm.at[pl.ds(r8, PIECE)],
                                          wuk_v.at[pl.ds(r8, PIECE)],
                                          sem_side.at[2]).start(priority=0)
                    pltpu.make_async_copy(wuv_hbm.at[pl.ds(r8, PIECE)],
                                          wuv_v.at[pl.ds(r8, PIECE)],
                                          sem_side.at[3]).start(priority=1)

        def body(p, carry):
            pair(p, True)
            return carry

        lax.fori_loop(0, 8, body, 0)
        pair(8, False)

    rows8 = lax.broadcasted_iota(jnp.int32, (8, DH), 0)

    def qk_softmax(it):
        slot = it % 2
        g, b, c = coords(it)
        q8 = q8_v[g * NB + b]
        s = None
        for j in range(HG):
            lhs = jnp.where(rows8 == j, q8, 0.0).astype(BF16)
            d = lax.dot_general(lhs, kbuf[slot, j], NT, preferred_element_type=F32)
            s = d if s is None else s + d
        first = c == 0
        m_old = jnp.where(first, -jnp.inf, ma_v[...])
        l_old = jnp.where(first, 0.0, la_v[...])
        m_new = jnp.maximum(m_old, jnp.max(s, axis=1, keepdims=True))
        alpha = jnp.exp((m_old - m_new) * SCALE)
        p = jnp.exp((s - m_new) * SCALE)
        l_new = l_old * alpha + jnp.sum(p, axis=1, keepdims=True)
        ma_v[...] = m_new
        la_v[...] = l_new
        pa_v[slot] = p.astype(BF16)
        al_v[slot] = alpha
        ll_v[slot] = l_new

    pltpu.make_async_copy(xa_hbm, xa_v, sem_x.at[0]).start()
    pltpu.make_async_copy(xb_hbm, xb_v, sem_x.at[1]).start()

    issue_wide(wq_hbm, wq_v, sem_wq.at[0], 0, 18)
    issue_kv(k_hbm, kbuf, (sem_k.at[0],) * 2, 0, 0)

    ma_v[...] = jnp.zeros(ma_v.shape, F32)
    la_v[...] = jnp.zeros(la_v.shape, F32)
    acca_v[...] = jnp.zeros(acca_v.shape, F32)
    o_v[...] = jnp.zeros(o_v.shape, F32)
    outa_v[...] = jnp.zeros(outa_v.shape, F32)
    x8_v[...] = jnp.zeros(x8_v.shape, F32)
    _wait(xa_v, sem_x.at[0])
    x8_v[0:NB, 0:DM] = xa_v[...].astype(F32)
    _wait(wq_v, sem_wq.at[0])
    qa = jnp.dot(x8_v[:, 0:DM].astype(BF16), wq_v[...], preferred_element_type=F32)
    qa = qa.astype(BF16).astype(F32)
    for g in range(NG):
        for b in range(NB):
            t = jnp.zeros((8, DH), F32)
            for j in range(HG):
                h = g * HG + j
                row = jnp.broadcast_to(qa[b:b + 1, h * DH:(h + 1) * DH], (8, DH))
                t = jnp.where(rows8 == j, row, t)
            q8_v[g * NB + b] = t

    def head_mask():
        r = lax.broadcasted_iota(jnp.int32, (128, CHUNK), 0)
        c = lax.broadcasted_iota(jnp.int32, (128, CHUNK), 1)
        return (r & 31) == (c & 31)

    def scatter_o(g, b, o):
        for j in range(HG):
            row = jnp.broadcast_to(o[j:j + 1, :], (8, DH))
            o_v[g * HG + j] = jnp.where(rows8 == b, row, o_v[g * HG + j])

    def project_group(g):
        lhs = jnp.concatenate([o_v[g * HG + j] for j in range(HG)], axis=1).astype(BF16)
        outa_v[...] += lax.dot_general(lhs, wo_v[:, g * HG * DH:(g + 1) * HG * DH], NT,
                                       preferred_element_type=F32)

    def step(i, carry):
        slot = (i + 2) % 2
        nxt = 1 - slot

        @pl.when(i + 2 < NIT)
        def _():
            issue_kv(k_hbm, kbuf, (sem_k.at[slot],) * 2, i + 2, slot)

        _wait(kbuf.at[nxt], sem_k.at[nxt])
        qk_softmax(i + 1)

        @pl.when(i + 1 < NIT - 2)
        def _():
            issue_kv(v_hbm, vbuf, (sem_v.at[nxt],) * 2, i + 1, nxt)

        @pl.when(i + 1 == NIT - 2)
        def _():
            issue_kv(v_hbm, vbuf, (sem_vp.at[0], sem_vp.at[1]), NIT - 2, (NIT - 2) % 2)

        @pl.when(i + 1 == NIT - 1)
        def _():
            issue_v_last(NIT - 1, (NIT - 1) % 2)

        @pl.when(jnp.logical_and(i >= 0, i < NIT - 2))
        def _():
            g, b, c = coords(i)
            _wait(vbuf.at[slot], sem_v.at[slot])
            p = pa_v[slot]
            pv = None
            for j in range(HG):
                d = jnp.dot(p, vbuf[slot, j], preferred_element_type=F32)
                d = jnp.where(rows8 == j, d, 0.0)
                pv = d if pv is None else pv + d
            acc = jnp.where(c == 0, 0.0, acca_v[...] * al_v[slot]) + pv
            acca_v[...] = acc

            @pl.when(c == NC - 1)
            def _():
                scatter_o(g, b, acc / ll_v[slot])

        @pl.when(jnp.logical_and(i >= 0, i < 8))
        def _():
            issue_ckv(i)

        @pl.when(jnp.logical_and(i >= 8, i < 16))
        def _():
            issue_weights(i - 8)

        @pl.when(jnp.logical_and(i >= 16, i < 18))
        def _():
            issue_wide(wo_hbm, wo_v, sem_side.at[5], (i - 16) * 9, (i - 15) * 9)

        for gg in range(NG - 1):
            @pl.when(i == (gg + 1) * NB * NC + 5)
            def _():
                if gg == 0:
                    _wait(wo_v, sem_side.at[5])
                project_group(gg)

        @pl.when(i == NIT - NC)
        def _():
            project_group(NG - 1)

        def job_range(s0, n):
            return jnp.logical_and(i >= s0, i < s0 + n)

        @pl.when(i == J_INIT)
        def _():
            prow = lax.broadcasted_iota(jnp.int32, (128, CHUNK), 0)
            pcol = lax.broadcasted_iota(jnp.int32, (128, CHUNK), 1)
            p_v[...] = jnp.where((pcol >> 5) == prow, 1.0, 0.0).astype(BF16)
            outb_v[...] = jnp.zeros(outb_v.shape, F32)
            qb_v[...] = jnp.zeros(qb_v.shape, F32)
            ctx_v[...] = jnp.zeros(ctx_v.shape, F32)
            wqb_v[pl.ds(DM * NH, N_B1 * CHUNK - DM * NH), :] = jnp.zeros(
                (N_B1 * CHUNK - DM * NH, DH), BF16)
            _wait(xb_v, sem_x.at[1])
            x8_v[0:NB, 0:DM] = xb_v[...].astype(F32)
            for cc in range(N_B1):
                xbc_v[cc] = x8_v[:, cc * 128:(cc + 1) * 128].astype(BF16)

        @pl.when(i == J_B1)
        def _():
            _wait(wqb_v.at[pl.ds(0, DM * NH)], sem_side.at[1])

        @pl.when(job_range(J_B1, N_B1))
        def _():
            cc = i - J_B1
            r0 = pl.multiple_of(cc * CHUNK, CHUNK)
            y = jnp.dot(xbc_v[cc], p_v[...], preferred_element_type=F32)
            yb = jnp.broadcast_to(y[0:NB][:, None, :], (NB, NH, CHUNK)).reshape(128, CHUNK)
            x = jnp.where(head_mask(), yb, 0.0).astype(BF16)
            qb_v[...] += jnp.dot(x, wqb_v[pl.ds(r0, CHUNK), :], preferred_element_type=F32)

        @pl.when(i == J_B2)
        def _():
            _wait(wuk_v, sem_side.at[2])

        @pl.when(job_range(J_B2, N_B2))
        def _():
            cc = i - J_B2
            r0 = pl.multiple_of(cc * CHUNK, CHUNK)
            gq = lax.dot_general(qb_v[...].astype(BF16), wuk_v[pl.ds(r0, CHUNK), :], NT,
                                 preferred_element_type=F32)
            gm = jnp.where(head_mask(), gq, 0.0).astype(BF16)
            qabs_v[cc] = lax.dot_general(gm, p_v[...], NT,
                                         preferred_element_type=F32).astype(BF16)

        @pl.when(i == J_B3)
        def _():
            _wait(ckv_v, sem_side.at[0])

        @pl.when(job_range(J_B3, N_B3))
        def _():
            n = i - J_B3
            bb = n // 4
            cc = n % 4
            r0 = pl.multiple_of(n * CKV_ROWS, CKV_ROWS)
            q0 = pl.multiple_of(bb * NH, NH)
            qq = jnp.concatenate([qabs_v[k, pl.ds(q0, NH), :] for k in range(4)], axis=1)
            kv = ckv_v[pl.ds(r0, CKV_ROWS), :]
            sb = lax.dot_general(qq, kv, NT, preferred_element_type=F32)

            @pl.when(cc == 0)
            def _():
                m_v[...] = jnp.full(m_v.shape, -jnp.inf, F32)
                l_v[...] = jnp.zeros(l_v.shape, F32)
                acc_v[...] = jnp.zeros(acc_v.shape, F32)

            m_old = m_v[...]
            m_new = jnp.maximum(m_old, jnp.max(sb, axis=1, keepdims=True))
            al = jnp.exp((m_old - m_new) * SCALE)
            pb = jnp.exp((sb - m_new) * SCALE)
            l_b = l_v[...] * al + jnp.sum(pb, axis=1, keepdims=True)
            accb = acc_v[...] * al + jnp.dot(pb.astype(BF16), kv, preferred_element_type=F32)
            m_v[...] = m_new
            l_v[...] = l_b
            acc_v[...] = accb

            @pl.when(cc == 3)
            def _():
                cl = (accb / l_b).astype(BF16)
                for k in range(4):
                    cl_v[k, pl.ds(q0, NH), :] = cl[:, k * 128:(k + 1) * 128]

        @pl.when(i == J_B4)
        def _():
            _wait(wuv_v, sem_side.at[3])

        @pl.when(job_range(J_B4, N_B4))
        def _():
            cc = i - J_B4
            r0 = pl.multiple_of(cc * CHUNK, CHUNK)
            y = jnp.dot(cl_v[cc], p_v[...], preferred_element_type=F32)
            e = jnp.where(head_mask(), y, 0.0).astype(BF16)
            ctx_v[...] += jnp.dot(e, wuv_v[pl.ds(r0, CHUNK), :], preferred_element_type=F32)

        @pl.when(i == J_B5)
        def _():
            _wait(wob_v, sem_side.at[4])
            r = lax.broadcasted_iota(jnp.int32, (NH * 8, 128), 0)
            cc = lax.broadcasted_iota(jnp.int32, (NH * 8, 128), 1)
            valid = (r & 7) < NB
            perm = jnp.where(jnp.logical_and(valid, cc == (r & 7) * NH + (r >> 3)), 1.0, 0.0)
            cp = jnp.dot(perm.astype(BF16), ctx_v[...].astype(BF16), preferred_element_type=F32)
            for hh in range(NH):
                cp_v[hh] = cp[hh * 8:(hh + 1) * 8].astype(BF16)

        @pl.when(job_range(J_B5, N_B5))
        def _():
            gb = i - J_B5
            r0 = pl.multiple_of(gb * WOB_ROWS, WOB_ROWS)
            accb = outb_v[...]
            for hh in range(8):
                rr = pl.multiple_of(r0 + hh * DM, 64)
                accb += lax.dot_general(cp_v[gb * 8 + hh], wob_v[pl.ds(rr, DM), :], NT,
                                        preferred_element_type=F32)
            outb_v[...] = accb

        return carry

    lax.fori_loop(-1, NIT - 1, step, 0)

    g = NG - 1
    s2 = (NIT - 2) % 2
    s3 = (NIT - 1) % 2
    p2 = pa_v[s2]
    p3 = pa_v[s3]
    a3 = al_v[s3]
    inv_l = 1.0 / ll_v[s3]
    base = acca_v[...] * al_v[s2]
    rows_m = lax.broadcasted_iota(jnp.int32, (8, DM), 0)
    acc2 = {}

    def pv2(parity):
        for j in range(parity, HG, 2):
            _wait(vbuf.at[s2, j], sem_vp.at[parity])
        for j in range(parity, HG, 2):
            acc2[j] = (base + jnp.dot(p2, vbuf[s2, j], preferred_element_type=F32)) * a3

    def last_head(j):
        _wait(vbuf.at[s3, j], sem_vl.at[j])
        o = (acc2[j] + jnp.dot(p3, vbuf[s3, j], preferred_element_type=F32)) * inv_l
        h = g * HG + j
        d = lax.dot_general(o.astype(BF16), wo_v[:, h * DH:(h + 1) * DH], NT,
                            preferred_element_type=F32)
        return jnp.where(rows_m == j, d, 0.0)

    pv2(0)
    part = last_head(LAST_Q0[0]) + last_head(LAST_Q0[1]) + last_head(LAST_Q0[2])
    pv2(1)
    part = part + last_head(LAST_Q0[3])
    for j in LAST_Q1[:-1]:
        part = part + last_head(j)
    part_row = jnp.broadcast_to(jnp.sum(part, axis=0, keepdims=True), (8, DM))
    outa = outa_v[...] + jnp.where(rows_m == NB - 1, part_row, 0.0)
    outa = outa + last_head(LAST_Q1[-1])
    res = jnp.concatenate([outa, outb_v[...]], axis=1)
    out_ref[...] = res[0:NB].astype(BF16)


@jax.jit
def pallas_concat_heads__mha_block_cached__compressed_kv_cla__decode_kernel(
    A_x: jax.Array,
    A_k_cache: jax.Array,
    A_v_cache: jax.Array,
    A_wq: jax.Array,
    A_wo: jax.Array,
    B_x: jax.Array,
    B_c_kv: jax.Array,
    B_w_q: jax.Array,
    B_w_uk: jax.Array,
    B_w_uv: jax.Array,
    B_w_o: jax.Array,
):
    ckv2 = B_c_kv.reshape(NB * SK, DC)
    wqb2 = B_w_q.reshape(DM * NH, DH)
    wuk2 = B_w_uk.reshape(DC * NH, DH)
    wuv2 = B_w_uv.reshape(DC * NH, DH)
    wob2 = B_w_o.transpose(0, 2, 1).reshape(NH * DM, DH)
    wo_t = A_wo.T
    xa2 = A_x.reshape(NB, DM)
    xb2 = B_x.reshape(NB, DM)

    vm = pltpu.VMEM
    n_b1_rows = N_B1 * CHUNK
    scratch = [
        vm((NB, DM), BF16),
        vm((NB, DM), BF16),
        vm((2, HG, ROWS, DH), BF16),
        vm((2, HG, ROWS, DH), BF16),
        vm((DM, NH * DH), BF16),
        vm((DM, NH * DH), BF16),
        vm((n_b1_rows, DH), BF16),
        vm((DC * NH, DH), BF16),
        vm((DC * NH, DH), BF16),
        vm((NH * DM, DH), BF16),
        vm((NB * SK, DC), BF16),
        vm((128, CHUNK), BF16),
        vm((8, N_B1 * 128), F32),
        vm((N_B1, 8, 128), BF16),
        vm((NG * NB, 8, DH), F32),
        vm((8, 1), F32),
        vm((8, 1), F32),
        vm((2, 8, ROWS), BF16),
        vm((2, 8, 1), F32),
        vm((2, 8, 1), F32),
        vm((8, DH), F32),
        vm((NH, 8, DH), F32),
        vm((128, DH), F32),
        vm((4, 128, 128), BF16),
        vm((NH, 1), F32),
        vm((NH, 1), F32),
        vm((NH, DC), F32),
        vm((4, 128, 128), BF16),
        vm((128, DH), F32),
        vm((NH, 8, DH), BF16),
        vm((8, DM), F32),
        vm((8, DM), F32),
        pltpu.SemaphoreType.DMA((2,)),
        pltpu.SemaphoreType.DMA((1,)),
        pltpu.SemaphoreType.DMA((2,)),
        pltpu.SemaphoreType.DMA((2,)),
        pltpu.SemaphoreType.DMA((2,)),
        pltpu.SemaphoreType.DMA((HG,)),
        pltpu.SemaphoreType.DMA((6,)),
    ]
    out = pl.pallas_call(
        _kernel,
        out_shape=jax.ShapeDtypeStruct((NB, 2 * DM), BF16),
        in_specs=[pl.BlockSpec(memory_space=pl.ANY)] * 11,
        out_specs=pl.BlockSpec(memory_space=pltpu.VMEM),
        scratch_shapes=scratch,
        compiler_params=pltpu.CompilerParams(vmem_limit_bytes=110 * 1024 * 1024,
                                             disable_semaphore_checks=True),
    )(xa2, A_k_cache, A_v_cache, A_wq, wo_t, xb2, ckv2, wqb2, wuk2, wuv2, wob2)
    return out.reshape(NB, 1, 2 * DM)
```

```python
import jax
import jax.numpy as jnp
from jax import lax
import jax.experimental.pallas as pl
import jax.experimental.pallas.tpu as pltpu

F32 = jnp.float32
BF16 = jnp.bfloat16

NB = 4
NH = 32
SK = 4096
DH = 128
DM = 576
DC = 512
SCALE = DH ** -0.5

HG = 8
NG = NH // HG
ROWS = 1024
NC = SK // ROWS
NIT = NG * NB * NC
PIECE = 128
NPIECE = ROWS // PIECE

CHUNK = 4096
CKV_ROWS = 1024
WOB_ROWS = 8 * DM

J_INIT = 1
J_B1, N_B1 = 18, 5
J_B2, N_B2 = J_B1 + N_B1, 4
J_B3, N_B3 = J_B2 + N_B2, 16
J_B4, N_B4 = J_B3 + N_B3, 4
J_B5, N_B5 = J_B4 + N_B4, 4

NT = (((1,), (1,)), ((), ()))

LAST_Q0 = (0, 2, 4, 6)
LAST_Q1 = (1, 5, 7, 3)
PARITY_POS = tuple((j % 2) * (HG // 2) + j // 2 for j in range(HG))


def _wait(buf_view, sem):
    pltpu.make_async_copy(buf_view, buf_view, sem).wait()


def _kernel(xa_hbm, k_hbm, v_hbm, wq_hbm, wo_hbm, xb_hbm, ckv_hbm, wqb_hbm, wuk_hbm, wuv_hbm,
            wob_hbm, out_ref,
            xa_v, xb_v, kbuf, vbuf, wq_v, wo_v, wqb_v, wuk_v, wuv_v, wob_v, ckv_v,
            p_v, x8_v, xbc_v, q8_v, ma_v, la_v, pa_v, al_v, ll_v, acca_v, o_v,
            qb_v, qabs_v, m_v, l_v, acc_v, cl_v, ctx_v, cp_v, outa_v, outb_v,
            sem_x, sem_wq, sem_k, sem_v, sem_vp, sem_vl, sem_side):

    def coords(it):
        return it // (NB * NC), (it // NC) % NB, it % NC

    def issue_kv(src, dst, sems, it, slot, pos=tuple(range(HG))):
        g, b, c = coords(it)

        def body(r, carry):
            r0 = pl.multiple_of(r * PIECE, PIECE)
            s0 = pl.multiple_of(c * ROWS + r0, PIECE)
            for j in range(HG):
                pltpu.make_async_copy(src.at[b, g * HG + j, pl.ds(s0, PIECE)],
                                      dst.at[slot, pos[j], pl.ds(r0, PIECE)],
                                      sems[j % 2]).start(priority=j % 2)
            return carry

        lax.fori_loop(0, NPIECE, body, 0)

    def issue_v_last(it, slot):
        g, b, c = coords(it)
        q0 = [(j, r) for j in LAST_Q0 for r in range(NPIECE)]
        q1 = [(j, r) for j in LAST_Q1 for r in range(NPIECE)]
        for pair in zip(q0, q1):
            for prio, (j, r) in enumerate(pair):
                pltpu.make_async_copy(v_hbm.at[b, g * HG + j, pl.ds(c * ROWS + r * PIECE, PIECE)],
                                      vbuf.at[slot, j, pl.ds(r * PIECE, PIECE)],
                                      sem_vl.at[j]).start(priority=prio)

    def issue_wide(src, dst, sem, t0, t1):
        def body(t, carry):
            for s in range(8):
                rr = pl.multiple_of((s * 9 + t // 2) * 8, 8)
                cc = pl.multiple_of((t % 2) * 2048, 2048)
                pltpu.make_async_copy(src.at[pl.ds(rr, 8), pl.ds(cc, 2048)],
                                      dst.at[pl.ds(rr, 8), pl.ds(cc, 2048)],
                                      sem).start(priority=s % 2)
            return carry

        lax.fori_loop(t0, t1, body, 0)

    def issue_ckv(t):
        def body(p, carry):
            for s in range(8):
                r0 = pl.multiple_of(s * 2048 + t * 256 + p * 32, 32)
                pltpu.make_async_copy(ckv_hbm.at[pl.ds(r0, 32)], ckv_v.at[pl.ds(r0, 32)],
                                      sem_side.at[0]).start(priority=s % 2)
            return carry

        lax.fori_loop(0, 8, body, 0)

    def issue_weights(t):
        def pair(p, with_small):
            for half in range(2):
                r9 = pl.multiple_of(half * (72 * PIECE) + (t * 9 + p) * PIECE, PIECE)
                pltpu.make_async_copy(wqb_hbm.at[pl.ds(r9, PIECE)], wqb_v.at[pl.ds(r9, PIECE)],
                                      sem_side.at[1]).start(priority=0)
                pltpu.make_async_copy(wob_hbm.at[pl.ds(r9, PIECE)], wob_v.at[pl.ds(r9, PIECE)],
                                      sem_side.at[4]).start(priority=1)
                if with_small:
                    r8 = pl.multiple_of(half * (64 * PIECE) + (t * 8 + p) * PIECE, PIECE)
                    pltpu.make_async_copy(wuk_hbm.at[pl.ds(r8, PIECE)],
                                          wuk_v.at[pl.ds(r8, PIECE)],
                                          sem_side.at[2]).start(priority=0)
                    pltpu.make_async_copy(wuv_hbm.at[pl.ds(r8, PIECE)],
                                          wuv_v.at[pl.ds(r8, PIECE)],
                                          sem_side.at[3]).start(priority=1)

        def body(p, carry):
            pair(p, True)
            return carry

        lax.fori_loop(0, 8, body, 0)
        pair(8, False)

    rows8 = lax.broadcasted_iota(jnp.int32, (8, DH), 0)

    def qk_softmax(it):
        slot = it % 2
        g, b, c = coords(it)
        q8 = q8_v[g * NB + b]
        s = None
        for j in range(HG):
            lhs = jnp.where(rows8 == j, q8, 0.0).astype(BF16)
            d = lax.dot_general(lhs, kbuf[slot, j], NT, preferred_element_type=F32)
            s = d if s is None else s + d
        first = c == 0
        m_old = jnp.where(first, -jnp.inf, ma_v[...])
        l_old = jnp.where(first, 0.0, la_v[...])
        m_new = jnp.maximum(m_old, jnp.max(s, axis=1, keepdims=True))
        alpha = jnp.exp((m_old - m_new) * SCALE)
        p = jnp.exp((s - m_new) * SCALE)
        l_new = l_old * alpha + jnp.sum(p, axis=1, keepdims=True)
        ma_v[...] = m_new
        la_v[...] = l_new
        pa_v[slot] = p.astype(BF16)
        al_v[slot] = alpha
        ll_v[slot] = l_new

    pltpu.make_async_copy(xa_hbm, xa_v, sem_x.at[0]).start()
    pltpu.make_async_copy(xb_hbm, xb_v, sem_x.at[1]).start()

    issue_wide(wq_hbm, wq_v, sem_wq.at[0], 0, 18)
    issue_kv(k_hbm, kbuf, (sem_k.at[0],) * 2, 0, 0)

    ma_v[...] = jnp.zeros(ma_v.shape, F32)
    la_v[...] = jnp.zeros(la_v.shape, F32)
    acca_v[...] = jnp.zeros(acca_v.shape, F32)
    o_v[...] = jnp.zeros(o_v.shape, F32)
    outa_v[...] = jnp.zeros(outa_v.shape, F32)
    x8_v[...] = jnp.zeros(x8_v.shape, F32)
    _wait(xa_v, sem_x.at[0])
    x8_v[0:NB, 0:DM] = xa_v[...].astype(F32)
    _wait(wq_v, sem_wq.at[0])
    qa = jnp.dot(x8_v[:, 0:DM].astype(BF16), wq_v[...], preferred_element_type=F32)
    qa = qa.astype(BF16).astype(F32)
    for g in range(NG):
        for b in range(NB):
            t = jnp.zeros((8, DH), F32)
            for j in range(HG):
                h = g * HG + j
                row = jnp.broadcast_to(qa[b:b + 1, h * DH:(h + 1) * DH], (8, DH))
                t = jnp.where(rows8 == j, row, t)
            q8_v[g * NB + b] = t

    def head_mask():
        r = lax.broadcasted_iota(jnp.int32, (128, CHUNK), 0)
        c = lax.broadcasted_iota(jnp.int32, (128, CHUNK), 1)
        return (r & 31) == (c & 31)

    def scatter_o(g, b, o):
        for j in range(HG):
            row = jnp.broadcast_to(o[j:j + 1, :], (8, DH))
            o_v[g * HG + j] = jnp.where(rows8 == b, row, o_v[g * HG + j])

    def project_group(g):
        lhs = jnp.concatenate([o_v[g * HG + j] for j in range(HG)], axis=1).astype(BF16)
        outa_v[...] += lax.dot_general(lhs, wo_v[:, g * HG * DH:(g + 1) * HG * DH], NT,
                                       preferred_element_type=F32)

    def step(i, carry):
        slot = (i + 2) % 2
        nxt = 1 - slot

        @pl.when(i + 2 < NIT)
        def _():
            issue_kv(k_hbm, kbuf, (sem_k.at[slot],) * 2, i + 2, slot)

        _wait(kbuf.at[nxt], sem_k.at[nxt])
        qk_softmax(i + 1)

        @pl.when(i + 1 < NIT - 2)
        def _():
            issue_kv(v_hbm, vbuf, (sem_v.at[nxt],) * 2, i + 1, nxt)

        @pl.when(i + 1 == NIT - 2)
        def _():
            issue_kv(v_hbm, vbuf, (sem_vp.at[0], sem_vp.at[1]), NIT - 2, (NIT - 2) % 2,
                     pos=PARITY_POS)

        @pl.when(i + 1 == NIT - 1)
        def _():
            issue_v_last(NIT - 1, (NIT - 1) % 2)

        @pl.when(jnp.logical_and(i >= 0, i < NIT - 2))
        def _():
            g, b, c = coords(i)
            _wait(vbuf.at[slot], sem_v.at[slot])
            p = pa_v[slot]
            pv = None
            for j in range(HG):
                d = jnp.dot(p, vbuf[slot, j], preferred_element_type=F32)
                d = jnp.where(rows8 == j, d, 0.0)
                pv = d if pv is None else pv + d
            acc = jnp.where(c == 0, 0.0, acca_v[...] * al_v[slot]) + pv
            acca_v[...] = acc

            @pl.when(c == NC - 1)
            def _():
                scatter_o(g, b, acc / ll_v[slot])

        @pl.when(jnp.logical_and(i >= 0, i < 8))
        def _():
            issue_ckv(i)

        @pl.when(jnp.logical_and(i >= 8, i < 16))
        def _():
            issue_weights(i - 8)

        @pl.when(jnp.logical_and(i >= 16, i < 18))
        def _():
            issue_wide(wo_hbm, wo_v, sem_side.at[5], (i - 16) * 9, (i - 15) * 9)

        for gg in range(NG - 1):
            @pl.when(i == (gg + 1) * NB * NC + 5)
            def _():
                if gg == 0:
                    _wait(wo_v, sem_side.at[5])
                project_group(gg)

        @pl.when(i == NIT - NC)
        def _():
            project_group(NG - 1)

        def job_range(s0, n):
            return jnp.logical_and(i >= s0, i < s0 + n)

        @pl.when(i == J_INIT)
        def _():
            prow = lax.broadcasted_iota(jnp.int32, (128, CHUNK), 0)
            pcol = lax.broadcasted_iota(jnp.int32, (128, CHUNK), 1)
            p_v[...] = jnp.where((pcol >> 5) == prow, 1.0, 0.0).astype(BF16)
            outb_v[...] = jnp.zeros(outb_v.shape, F32)
            qb_v[...] = jnp.zeros(qb_v.shape, F32)
            ctx_v[...] = jnp.zeros(ctx_v.shape, F32)
            wqb_v[pl.ds(DM * NH, N_B1 * CHUNK - DM * NH), :] = jnp.zeros(
                (N_B1 * CHUNK - DM * NH, DH), BF16)
            _wait(xb_v, sem_x.at[1])
            x8_v[0:NB, 0:DM] = xb_v[...].astype(F32)
            for cc in range(N_B1):
                xbc_v[cc] = x8_v[:, cc * 128:(cc + 1) * 128].astype(BF16)

        @pl.when(i == J_B1)
        def _():
            _wait(wqb_v.at[pl.ds(0, DM * NH)], sem_side.at[1])

        @pl.when(job_range(J_B1, N_B1))
        def _():
            cc = i - J_B1
            r0 = pl.multiple_of(cc * CHUNK, CHUNK)
            y = jnp.dot(xbc_v[cc], p_v[...], preferred_element_type=F32)
            yb = jnp.broadcast_to(y[0:NB][:, None, :], (NB, NH, CHUNK)).reshape(128, CHUNK)
            x = jnp.where(head_mask(), yb, 0.0).astype(BF16)
            qb_v[...] += jnp.dot(x, wqb_v[pl.ds(r0, CHUNK), :], preferred_element_type=F32)

        @pl.when(i == J_B2)
        def _():
            _wait(wuk_v, sem_side.at[2])

        @pl.when(job_range(J_B2, N_B2))
        def _():
            cc = i - J_B2
            r0 = pl.multiple_of(cc * CHUNK, CHUNK)
            gq = lax.dot_general(qb_v[...].astype(BF16), wuk_v[pl.ds(r0, CHUNK), :], NT,
                                 preferred_element_type=F32)
            gm = jnp.where(head_mask(), gq, 0.0).astype(BF16)
            qabs_v[cc] = lax.dot_general(gm, p_v[...], NT,
                                         preferred_element_type=F32).astype(BF16)

        @pl.when(i == J_B3)
        def _():
            _wait(ckv_v, sem_side.at[0])

        @pl.when(job_range(J_B3, N_B3))
        def _():
            n = i - J_B3
            bb = n // 4
            cc = n % 4
            r0 = pl.multiple_of(n * CKV_ROWS, CKV_ROWS)
            q0 = pl.multiple_of(bb * NH, NH)
            qq = jnp.concatenate([qabs_v[k, pl.ds(q0, NH), :] for k in range(4)], axis=1)
            kv = ckv_v[pl.ds(r0, CKV_ROWS), :]
            sb = lax.dot_general(qq, kv, NT, preferred_element_type=F32)

            @pl.when(cc == 0)
            def _():
                m_v[...] = jnp.full(m_v.shape, -jnp.inf, F32)
                l_v[...] = jnp.zeros(l_v.shape, F32)
                acc_v[...] = jnp.zeros(acc_v.shape, F32)

            m_old = m_v[...]
            m_new = jnp.maximum(m_old, jnp.max(sb, axis=1, keepdims=True))
            al = jnp.exp((m_old - m_new) * SCALE)
            pb = jnp.exp((sb - m_new) * SCALE)
            l_b = l_v[...] * al + jnp.sum(pb, axis=1, keepdims=True)
            accb = acc_v[...] * al + jnp.dot(pb.astype(BF16), kv, preferred_element_type=F32)
            m_v[...] = m_new
            l_v[...] = l_b
            acc_v[...] = accb

            @pl.when(cc == 3)
            def _():
                cl = (accb / l_b).astype(BF16)
                for k in range(4):
                    cl_v[k, pl.ds(q0, NH), :] = cl[:, k * 128:(k + 1) * 128]

        @pl.when(i == J_B4)
        def _():
            _wait(wuv_v, sem_side.at[3])

        @pl.when(job_range(J_B4, N_B4))
        def _():
            cc = i - J_B4
            r0 = pl.multiple_of(cc * CHUNK, CHUNK)
            y = jnp.dot(cl_v[cc], p_v[...], preferred_element_type=F32)
            e = jnp.where(head_mask(), y, 0.0).astype(BF16)
            ctx_v[...] += jnp.dot(e, wuv_v[pl.ds(r0, CHUNK), :], preferred_element_type=F32)

        @pl.when(i == J_B5)
        def _():
            _wait(wob_v, sem_side.at[4])
            r = lax.broadcasted_iota(jnp.int32, (NH * 8, 128), 0)
            cc = lax.broadcasted_iota(jnp.int32, (NH * 8, 128), 1)
            valid = (r & 7) < NB
            perm = jnp.where(jnp.logical_and(valid, cc == (r & 7) * NH + (r >> 3)), 1.0, 0.0)
            cp = jnp.dot(perm.astype(BF16), ctx_v[...].astype(BF16), preferred_element_type=F32)
            for hh in range(NH):
                cp_v[hh] = cp[hh * 8:(hh + 1) * 8].astype(BF16)

        @pl.when(job_range(J_B5, N_B5))
        def _():
            gb = i - J_B5
            r0 = pl.multiple_of(gb * WOB_ROWS, WOB_ROWS)
            accb = outb_v[...]
            for hh in range(8):
                rr = pl.multiple_of(r0 + hh * DM, 64)
                accb += lax.dot_general(cp_v[gb * 8 + hh], wob_v[pl.ds(rr, DM), :], NT,
                                        preferred_element_type=F32)
            outb_v[...] = accb

        return carry

    lax.fori_loop(-1, NIT - 1, step, 0)

    g = NG - 1
    s2 = (NIT - 2) % 2
    s3 = (NIT - 1) % 2
    p2 = pa_v[s2]
    p3 = pa_v[s3]
    a3 = al_v[s3]
    inv_l = 1.0 / ll_v[s3]
    base = acca_v[...] * al_v[s2]
    rows_m = lax.broadcasted_iota(jnp.int32, (8, DM), 0)
    acc2 = {}

    def pv2(parity):
        _wait(vbuf.at[s2, pl.ds(parity * (HG // 2), HG // 2)], sem_vp.at[parity])
        for j in range(parity, HG, 2):
            acc2[j] = (base + jnp.dot(p2, vbuf[s2, PARITY_POS[j]],
                                      preferred_element_type=F32)) * a3

    def last_head(j):
        _wait(vbuf.at[s3, j], sem_vl.at[j])
        o = (acc2[j] + jnp.dot(p3, vbuf[s3, j], preferred_element_type=F32)) * inv_l
        h = g * HG + j
        d = lax.dot_general(o.astype(BF16), wo_v[:, h * DH:(h + 1) * DH], NT,
                            preferred_element_type=F32)
        return jnp.where(rows_m == j, d, 0.0)

    pv2(0)
    part = last_head(LAST_Q0[0]) + last_head(LAST_Q0[1]) + last_head(LAST_Q0[2])
    pv2(1)
    part = part + last_head(LAST_Q0[3])
    for j in LAST_Q1[:-1]:
        part = part + last_head(j)
    part_row = jnp.broadcast_to(jnp.sum(part, axis=0, keepdims=True), (8, DM))
    outa = outa_v[...] + jnp.where(rows_m == NB - 1, part_row, 0.0)
    outa = outa + last_head(LAST_Q1[-1])
    res = jnp.concatenate([outa, outb_v[...]], axis=1)
    out_ref[...] = res[0:NB].astype(BF16)


@jax.jit
def pallas_concat_heads__mha_block_cached__compressed_kv_cla__decode_kernel(
    A_x: jax.Array,
    A_k_cache: jax.Array,
    A_v_cache: jax.Array,
    A_wq: jax.Array,
    A_wo: jax.Array,
    B_x: jax.Array,
    B_c_kv: jax.Array,
    B_w_q: jax.Array,
    B_w_uk: jax.Array,
    B_w_uv: jax.Array,
    B_w_o: jax.Array,
):
    ckv2 = B_c_kv.reshape(NB * SK, DC)
    wqb2 = B_w_q.reshape(DM * NH, DH)
    wuk2 = B_w_uk.reshape(DC * NH, DH)
    wuv2 = B_w_uv.reshape(DC * NH, DH)
    wob2 = B_w_o.transpose(0, 2, 1).reshape(NH * DM, DH)
    wo_t = A_wo.T
    xa2 = A_x.reshape(NB, DM)
    xb2 = B_x.reshape(NB, DM)

    vm = pltpu.VMEM
    n_b1_rows = N_B1 * CHUNK
    scratch = [
        vm((NB, DM), BF16),
        vm((NB, DM), BF16),
        vm((2, HG, ROWS, DH), BF16),
        vm((2, HG, ROWS, DH), BF16),
        vm((DM, NH * DH), BF16),
        vm((DM, NH * DH), BF16),
        vm((n_b1_rows, DH), BF16),
        vm((DC * NH, DH), BF16),
        vm((DC * NH, DH), BF16),
        vm((NH * DM, DH), BF16),
        vm((NB * SK, DC), BF16),
        vm((128, CHUNK), BF16),
        vm((8, N_B1 * 128), F32),
        vm((N_B1, 8, 128), BF16),
        vm((NG * NB, 8, DH), F32),
        vm((8, 1), F32),
        vm((8, 1), F32),
        vm((2, 8, ROWS), BF16),
        vm((2, 8, 1), F32),
        vm((2, 8, 1), F32),
        vm((8, DH), F32),
        vm((NH, 8, DH), F32),
        vm((128, DH), F32),
        vm((4, 128, 128), BF16),
        vm((NH, 1), F32),
        vm((NH, 1), F32),
        vm((NH, DC), F32),
        vm((4, 128, 128), BF16),
        vm((128, DH), F32),
        vm((NH, 8, DH), BF16),
        vm((8, DM), F32),
        vm((8, DM), F32),
        pltpu.SemaphoreType.DMA((2,)),
        pltpu.SemaphoreType.DMA((1,)),
        pltpu.SemaphoreType.DMA((2,)),
        pltpu.SemaphoreType.DMA((2,)),
        pltpu.SemaphoreType.DMA((2,)),
        pltpu.SemaphoreType.DMA((HG,)),
        pltpu.SemaphoreType.DMA((6,)),
    ]
    out = pl.pallas_call(
        _kernel,
        out_shape=jax.ShapeDtypeStruct((NB, 2 * DM), BF16),
        in_specs=[pl.BlockSpec(memory_space=pl.ANY)] * 11,
        out_specs=pl.BlockSpec(memory_space=pltpu.VMEM),
        scratch_shapes=scratch,
        compiler_params=pltpu.CompilerParams(vmem_limit_bytes=110 * 1024 * 1024,
                                             disable_semaphore_checks=True),
    )(xa2, A_k_cache, A_v_cache, A_wq, wo_t, xb2, ckv2, wqb2, wuk2, wuv2, wob2)
    return out.reshape(NB, 1, 2 * DM)
```
